```python
import os as _os
_os.environ.setdefault("JAX_PLATFORMS", "cpu")
import jax
import jax.numpy as jnp

def _softmax(x, axis=-1):
    return jax.nn.softmax(x, axis=axis)
def _gelu(x):
    return jax.nn.gelu(x, approximate=True)
def _silu(x):
    return jax.nn.silu(x)
def _sigmoid(x):
    return jax.nn.sigmoid(x)
def _layernorm(x, axis=-1, eps=1e-5):
    m = jnp.mean(x, axis=axis, keepdims=True)
    v = jnp.var(x, axis=axis, keepdims=True)
    return (x - m) / jnp.sqrt(v + eps)
def _scatter_add(tgt, idx, src, axis=0):
    return tgt.at[idx].add(src)
def _segment_sum(src, seg, n):
    return jax.ops.segment_sum(src, seg, n)
class _Rng:
    def __init__(self, key):
        self._k = key
    def _next(self):
        self._k, sub = jax.random.split(self._k)
        return sub
    def normal(self, shape):
        return jax.random.normal(self._next(), shape, dtype=jnp.bfloat16)
    def randint(self, lo, hi, shape):
        return jax.random.randint(self._next(), shape, lo, hi, dtype=jnp.int32)
    def uniform(self, shape, lo=0.0, hi=1.0):
        return jax.random.uniform(self._next(), shape, jnp.bfloat16, lo, hi)
    def permutation(self, n):
        return jax.random.permutation(self._next(), n)


kernel_name = 'interleave_layers__sliding_block_cached__mixer_channel_mlp__decode'

def setup_inputs():
    _rng = _Rng(jax.random.key(int.from_bytes(__import__("os").urandom(4), "little")))
    _w = (lambda a: (lambda t: t.astype(jnp.bfloat16) if jnp.issubdtype(t.dtype, jnp.floating) else t)(jnp.asarray(a)))
    def _A_setup():
        B, Sq, D = 8, 1, 640
        Hq, Hkv, Sk, Dh = 32, 32, 4096, 128
        assert Hq % Hkv == 0, (Hq, Hkv)
        return {
            "x": _w((lambda *s: _rng.normal(s) * 0.05)(B, Sq, D)),
            "k_cache": _w((lambda *s: _rng.normal(s) * 1.6)(B, Hkv, Sk, Dh)),
            "v_cache": _w((lambda *s: _rng.normal(s) * 0.8)(B, Hkv, Sk, Dh)),
            "wq": _w((lambda *s: _rng.normal(s) * 1.6)(D, Hq * Dh) * (D ** -0.5)),
            "wo": _w((lambda *s: _rng.normal(s) * 0.8)(Hq * Dh, D) * ((Hq * Dh) ** -0.5)),
        }
    _A_in = _A_setup()

    def _B_setup():
        B, S, D, F = 8, 1, 640, 1728
        return {
            "x": _w((lambda *s: _rng.normal(s) * 0.05)(B, S, D)),
            "w1": _w((lambda *s: _rng.normal(s) * 0.4)(D, F) * (D ** -0.5)),
            "b1": _w((lambda *s: _rng.normal(s) * 0.4)(F)),
            "w2": _w((lambda *s: _rng.normal(s) * 0.4)(F, D) * (F ** -0.5)),
            "b2": _w((lambda *s: _rng.normal(s) * 0.2)(D)),
        }
    _B_in = _B_setup()

    return {
        "A_x": _A_in["x"],
        "A_k_cache": _A_in["k_cache"],
        "A_v_cache": _A_in["v_cache"],
        "A_wq": _A_in["wq"],
        "A_wo": _A_in["wo"],
        "B_x": _B_in["x"],
        "B_w1": _B_in["w1"],
        "B_b1": _B_in["b1"],
        "B_w2": _B_in["w2"],
        "B_b2": _B_in["b2"],
    }

def reference(A_x, A_k_cache, A_v_cache, A_wq, A_wo, B_x, B_w1, B_b1, B_w2, B_b2):
    def _A_ref(x, k_cache, v_cache, wq, wo):
        B, Sq, D = x.shape
        Hq, Dh = 32, 128
        Hkv, Sk = k_cache.shape[1], k_cache.shape[2]
        W = min(4096, max(256, Sk // 4))
        rep = Hq // Hkv
        q = (lambda x, *d: x.transpose(*d))((x @ wq).reshape(B, Sq, Hq, Dh), 0, 2, 1, 3)
        k = jnp.repeat(k_cache[:, :, Sk - W:, :], rep, axis=1)
        v = jnp.repeat(v_cache[:, :, Sk - W:, :], rep, axis=1)
        scores = jnp.einsum("bhqd,bhkd->bhqk", q, k) * (Dh ** -0.5)
        p = _softmax(scores, axis=-1)
        o = jnp.einsum("bhqk,bhkd->bhqd", p, v)
        return (lambda x, *d: x.transpose(*d))(o, 0, 2, 1, 3).reshape(B, Sq, Hq * Dh) @ wo

    def _B_ref(x, w1, b1, w2, b2):
        y = _layernorm(x, axis=-1)
        h = _gelu(jnp.einsum("bsd,df->bsf", y, w1) + b1)
        return jnp.einsum("bsf,fd->bsd", h, w2) + b2

    x = A_x
    x = x + _A_ref(_layernorm(x, axis=-1), A_k_cache, A_v_cache, A_wq, A_wo)
    x = x + _B_ref(_layernorm(x, axis=-1), B_w1, B_b1, B_w2, B_b2)
    x = x + _A_ref(_layernorm(x, axis=-1), A_k_cache, A_v_cache, A_wq, A_wo)
    x = x + _B_ref(_layernorm(x, axis=-1), B_w1, B_b1, B_w2, B_b2)
    return x
```

```python
import functools
import jax
import jax.numpy as jnp
from jax import lax
from jax.experimental import pallas as pl
from jax.experimental.pallas import tpu as pltpu

B, D, H, DH, SK, W, F = 8, 640, 32, 128, 4096, 1024, 1728
G = 8
NG = H // G
NP = 16
NT = (((1,), (1,)), ((), ()))
f32, bf16 = jnp.float32, jnp.bfloat16


def _ln(x):
    m = jnp.mean(x, axis=-1, keepdims=True)
    xc = x - m
    v = jnp.mean(xc * xc, axis=-1, keepdims=True)
    return xc * lax.rsqrt(v + 1e-5)


def make(LA=6, nr=128, nobc=True, compute=True, pts=4):
    NPAGE = B * NG * 2
    PR = W // nr
    PP = G * PR

    def kern(x_hbm, k_hbm, v_hbm, wq_hbm, wo_hbm, w1t_hbm, b1_hbm, w2_hbm, b2_hbm,
             o_ref, kv, wq, wo, w1t, w2, xs, b1s, b2s, psem, wsem):

        def issue(p, lo, hi):
            b = p // (2 * NG)
            g = (p // 2) % NG
            slot = p % NP
            def go(src):
                for i in range(lo, hi):
                    q = i % 2
                    hh = (i // 2) % G
                    r = (i // (2 * G)) + q * (PR // 2)
                    pltpu.make_async_copy(
                        src.at[b, g * G + hh, pl.ds(SK - W + r * nr, nr), :],
                        kv.at[slot, hh, pl.ds(r * nr, nr), :],
                        psem.at[slot]).start(priority=q)
            if isinstance(p, int):
                go((k_hbm, v_hbm)[p % 2])
            else:
                @pl.when((p < NPAGE) & (p % 2 == 0))
                def _():
                    go(k_hbm)
                @pl.when((p < NPAGE) & (p % 2 == 1))
                def _():
                    go(v_hbm)

        def wait_page(p):
            slot = p % NP
            pltpu.make_async_copy(kv.at[slot], kv.at[slot], psem.at[slot]).wait()

        i = 0
        for r in range(0, D, 8):
            for c in range(0, H * DH, 2048):
                pltpu.make_async_copy(wq_hbm.at[pl.ds(r, 8), pl.ds(c, 2048)], wq.at[pl.ds(r, 8), pl.ds(c, 2048)],
                                      wsem.at[0]).start(priority=i % 2)
                i += 1
        small = [pltpu.make_async_copy(x_hbm, xs, wsem.at[4]),
                 pltpu.make_async_copy(b1_hbm, b1s, wsem.at[5]),
                 pltpu.make_async_copy(b2_hbm, b2s, wsem.at[6])]
        for c in small:
            c.start()
        for src, dst, s, n in ((wo_hbm, wo, 1, H * DH), (w1t_hbm, w1t, 2, F), (w2_hbm, w2, 3, F)):
            step = 32
            half = n // 2
            for r in range(0, half, step):
                for q in range(2):
                    rr = r + q * half
                    pltpu.make_async_copy(src.at[pl.ds(rr, step), :], dst.at[pl.ds(rr, step), :],
                                          wsem.at[s]).start(priority=q)
        for p in range(LA):
            issue(p, 0, PP)
        pltpu.make_async_copy(wq, wq, wsem.at[0]).wait()
        pltpu.make_async_copy(wo, wo, wsem.at[1]).wait()
        pltpu.make_async_copy(w1t, w1t, wsem.at[2]).wait()
        pltpu.make_async_copy(w2, w2, wsem.at[3]).wait()
        for c in small:
            c.wait()

        row = lax.broadcasted_iota(jnp.int32, (8, DH), 0)
        rowd = lax.broadcasted_iota(jnp.int32, (8, D), 0)
        x_all = xs[...].astype(f32)
        b1 = b1s[...].astype(f32)[None, :]
        b2 = b2s[...].astype(f32)[None, :]
        scale = DH ** -0.5

        def layer(it, carry):
            x, res = carry
            b = it // 2
            x_in = jnp.broadcast_to(jnp.sum(jnp.where(rowd == b, x_all, 0.0), axis=0, keepdims=True), (8, D))
            x = jnp.where(it % 2 == 0, x_in, x)
            y = _ln(x).astype(bf16)

            def group(g, acc):
                p_issue = 4 * it + g + LA
                pk = b * (2 * NG) + 2 * g
                q4 = PP // pts
                issue(p_issue, 0, q4)
                if compute:
                    q = jnp.dot(y, wq[:, pl.ds(pl.multiple_of(g * G * DH, G * DH), G * DH)], preferred_element_type=f32)
                if pts >= 2:
                    issue(p_issue, q4, 2 * q4)

                @pl.when(it % 2 == 0)
                def _():
                    wait_page(pk)
                if compute:
                    s = None
                    for j in range(G):
                        qm = jnp.where(row == j, q[:, j * DH:(j + 1) * DH], 0.0).astype(bf16)
                        sj = lax.dot_general(qm, kv[pk % NP, j], NT, preferred_element_type=f32)
                        s = sj if s is None else s + sj
                    m = jnp.max(s, axis=-1, keepdims=True)
                    e = jnp.exp((s - m) * scale)
                    l = jnp.sum(e, axis=-1, keepdims=True)
                    pb = e.astype(bf16)
                    rl = 1.0 / l
                if pts >= 3:
                    issue(p_issue, 2 * q4, 3 * q4)

                @pl.when(it % 2 == 0)
                def _():
                    wait_page(pk + 1)
                if compute:
                    os = []
                    for j in range(G):
                        oj = jnp.dot(pb, kv[(pk + 1) % NP, j], preferred_element_type=f32)
                        os.append(jnp.where(row == j, oj * rl, 0.0).astype(bf16))
                if pts >= 4:
                    issue(p_issue, 3 * q4, 4 * q4)
                if compute:
                    o = jnp.concatenate(os, axis=1)
                    acc = acc + jnp.dot(o, wo[pl.ds(pl.multiple_of(g * G * DH, G * DH), G * DH), :],
                                        preferred_element_type=f32)
                return acc

            acc = lax.fori_loop(0, NG, group, jnp.zeros((8, D), f32))
            if compute:
                x = x + jnp.broadcast_to(jnp.sum(acc, axis=0, keepdims=True), (8, D))
                y2 = _ln(_ln(x)).astype(bf16)
                h = lax.dot_general(y2, w1t[...], NT, preferred_element_type=f32) + b1
                h = jax.nn.gelu(h, approximate=True).astype(bf16)
                x = x + jnp.dot(h, w2[...], preferred_element_type=f32) + b2
            res = jnp.where(rowd == b, x, res)
            return x, res

        _, res = lax.fori_loop(0, 2 * B, layer, (jnp.zeros((8, D), f32), jnp.zeros((8, D), f32)))
        o_ref[...] = res.astype(o_ref.dtype)

    def fn(A_x, A_k_cache, A_v_cache, A_wq, A_wo, B_x, B_w1, B_b1, B_w2, B_b2):
        hbm = pl.BlockSpec(memory_space=pltpu.HBM)
        out = pl.pallas_call(
            kern,
            in_specs=[hbm] * 9,
            out_specs=pl.BlockSpec(memory_space=pltpu.VMEM),
            out_shape=jax.ShapeDtypeStruct((B, D), bf16),
            scratch_shapes=[
                pltpu.VMEM((NP, G, W, DH), bf16),
                pltpu.VMEM((D, H * DH), bf16),
                pltpu.VMEM((H * DH, D), bf16),
                pltpu.VMEM((F, D), bf16),
                pltpu.VMEM((F, D), bf16),
                pltpu.VMEM((B, D), bf16),
                pltpu.VMEM((F,), bf16),
                pltpu.VMEM((D,), bf16),
                pltpu.SemaphoreType.DMA((NP,)),
                pltpu.SemaphoreType.DMA((7,)),
            ],
            compiler_params=pltpu.CompilerParams(vmem_limit_bytes=100 * 1024 * 1024, disable_bounds_checks=nobc),
        )(A_x.reshape(B, D), A_k_cache, A_v_cache, A_wq, A_wo, B_w1.T, B_b1, B_w2, B_b2)
        return out.reshape(B, 1, D)

    return jax.jit(fn)


_fn = make()


@jax.jit
def pallas_interleave_layers__sliding_block_cached__mixer_channel_mlp__decode_kernel(
    A_x, A_k_cache, A_v_cache, A_wq, A_wo, B_x, B_w1, B_b1, B_w2, B_b2):
    return _fn(A_x, A_k_cache, A_v_cache, A_wq, A_wo, B_x, B_w1, B_b1, B_w2, B_b2)
```

```python
import jax
import jax.numpy as jnp
from jax import lax
from jax.experimental import pallas as pl
from jax.experimental.pallas import tpu as pltpu

B, D, H, DH, SK, F = 8, 640, 32, 128, 4096, 1728
W = min(4096, max(256, SK // 4))
FP = 1792
DT = D // 128
G = 8
NG = H // G
NPAGE = B * NG
NK, NV = 4, 8
EPS = 1e-5
SCALE = DH ** -0.5 * 1.4426950408889634

PIECE_ROWS = (64, 192) * 4
HEAD_ORDER = (0, 4, 1, 5, 2, 6, 3, 7)
NS = len(PIECE_ROWS)

f32, bf16, u32 = jnp.float32, jnp.bfloat16, jnp.uint32


def tiles(v):
    return [v[:, i * 128:(i + 1) * 128] for i in range(v.shape[1] // 128)]


def tree(op, xs):
    xs = list(xs)
    while len(xs) > 1:
        xs = [op(*xs[i:i + 2]) if i + 1 < len(xs) else xs[i] for i in range(0, len(xs), 2)]
    return xs[0]


def lane_sum(v):
    return jnp.broadcast_to(jnp.sum(v, axis=1, keepdims=True), v.shape)


def lane_max(v):
    return jnp.broadcast_to(jnp.max(v, axis=1, keepdims=True), v.shape)


def row_sum(v):
    return jnp.broadcast_to(jnp.sum(v, axis=0, keepdims=True), v.shape)


def accum(acc, i, val):
    acc[i] = val if acc[i] is None else acc[i] + val


def pack(a, b=None):
    return pltpu.bitcast(jnp.concatenate([a, a if b is None else b], axis=0).astype(bf16), u32)


def unpack(w):
    return pltpu.bitcast(w, bf16)


def mxu_dot(lhs, w, half=0):
    lhs = jnp.concatenate([unpack(t) for t in lhs], axis=1)
    return jnp.dot(lhs, unpack(w), preferred_element_type=f32)[half * 8:half * 8 + 8]


def moments(xt):
    m = lane_sum(tree(jnp.add, xt)) * (1.0 / D)
    sq = lane_sum(tree(jnp.add, [t * t for t in xt])) * (1.0 / D)
    return m, jnp.maximum(sq - m * m, 0.0)


def gelu(x):
    c = 0.7978845608028654
    hx = 0.5 * x
    return hx + hx * jnp.tanh(x * (c + (c * 0.044715) * (x * x)))


def loop(n, body):
    lax.fori_loop(0, n, lambda i, c: (body(i), c)[1], 0)


class Weave:
    def __init__(self, always, lag_m, lag_v, lead=0.0):
        self.always, self.lag_m, self.lag_v, self.lead = always, lag_m, lag_v, lead
        self.vres, self.mres, self.fresh = [], [], False

    def tie_m(self, lhs):
        k = len(self.mres) - self.lag_m
        if k < 0 or self.vres[k] is None:
            return lhs
        return jnp.where(self.always, lhs, pltpu.bitcast(self.vres[k], u32))

    def tie_v(self, val):
        k = len(self.mres) - self.lag_v
        if k < 0 or not self.fresh:
            return val
        self.fresh = False
        return jnp.where(self.always, val, self.mres[k])

    def run(self, mxu, mxu_work, vpu, vpu_work):
        md = vd = 0
        last = None
        mxu_live, vpu_live = True, vpu_work > 0
        while mxu_live or vpu_live:
            if mxu_live and (not vpu_live or md / mxu_work <= -self.lead + (1 + self.lead) * vd / vpu_work):
                item = next(mxu, None)
                mxu_live = item is not None
                if mxu_live:
                    md += item[0]
                    self.vres.append(last)
                    self.mres.append(item[1])
                    self.fresh = True
            else:
                item = next(vpu, None)
                vpu_live = item is not None
                if vpu_live:
                    vd += item[0]
                    last = item[1]


JB = 4


def mlp(xt, refs, fm, weave, depth, feed=None):
    w1, w2, cs1, b1, b2, w1tf, w2f, b1col = refs
    m, var = moments(xt)
    r1 = lax.rsqrt(var + EPS)
    r = r1 * lax.rsqrt(var * r1 * r1 + EPS)
    xp = [pack(xt[i], xt[min(i + 1, DT - 1)]) for i in range(0, DT, 2)]
    xc = [t - m for t in xt]
    macc, vacc = [None] * DT, [None] * DT
    chunks = [(c, min(4, fm - c)) for c in range(0, fm, 4)]
    nj = max(F - fm * 128, 0) // 8

    def mxu():
        hs = {}

        def up(i):
            c0, n = chunks[i]
            a = None
            for kb in range(DT):
                u = mxu_dot([weave.tie_m(xp[kb // 2])], w1[kb * 64:(kb + 1) * 64, c0 * 128:(c0 + n) * 128], kb % 2)
                a = u if a is None else a + u
                yield 8 * n, u[:, 0:128]
            hs[i] = []
            for j, t in enumerate(tiles(a)):
                sl = slice((c0 + j) * 128, (c0 + j + 1) * 128)
                hs[i].append(pack(gelu((t - m * cs1[:, sl]) * r + b1[:, sl])))

        def down(i):
            c0, n = chunks[i]
            for nt in range(DT):
                u = mxu_dot([weave.tie_m(hs[i][0])] + hs[i][1:], w2[c0 * 64:(c0 + n) * 64, nt * 128:(nt + 1) * 128])
                accum(macc, nt, u)
                yield 8 * n, u

        for t in range(len(chunks) + depth):
            if t < len(chunks):
                if feed:
                    feed()
                yield from up(t)
            if t >= depth:
                yield from down(t - depth)

    def vpu():
        delay = 48
        col, part = {}, {}
        for step in range(nj + delay):
            if step < nj:
                blk, sub = divmod(step, JB)
                js = range(blk * JB, (blk + 1) * JB)
                for kb in range(DT):
                    if kb * JB // DT == sub:
                        x0 = weave.tie_v(xc[kb])
                        for j in js:
                            t = w1tf[j * 8:(j + 1) * 8, kb * 128:(kb + 1) * 128] * x0
                            part[j] = t if kb == 0 else part[j] + t
                        yield JB, part[j]
                if sub == JB - 1:
                    for j in js:
                        col[j] = lane_sum(part.pop(j))
            j = step - delay
            if j >= 0:
                h = weave.tie_v(gelu(col.pop(j) * r + b1col[j * 8:(j + 1) * 8, :]))
                for nt in range(DT):
                    accum(vacc, nt, w2f[j * 8:(j + 1) * 8, nt * 128:(nt + 1) * 128] * h)
                yield 5, vacc[DT - 1]

    weave.run(mxu(), fm * 80, vpu(), nj * 10)
    out = []
    for nt in range(DT):
        a = xt[nt] + b2[:, nt * 128:(nt + 1) * 128] + macc[nt]
        out.append(a if vacc[nt] is None else a + row_sum(vacc[nt]))
    return out


def attention(xt, refs, vheads, groups, weave):
    k_half, v_half, wq, wo, csq, ktf, vtf, wqtf, wof = refs
    row = lax.broadcasted_iota(jnp.int32, (8, DH), 0)
    m, var = moments(xt)
    c = lax.rsqrt(var + EPS) * SCALE
    xc = [t - m for t in xt]
    xp = [pack(xt[i], xt[min(i + 1, DT - 1)]) for i in range(0, DT, 2)]
    macc, vacc = [None] * DT, [None] * DT

    def mxu():
        q, p, o = {}, {}, {}

        def project(g):
            for c0 in range(0, len(groups[g]), 4):
                hs = groups[g][c0:c0 + 4]
                a = None
                for kb in range(DT):
                    w = jnp.concatenate([wq[kb * 64:(kb + 1) * 64, h * 128:(h + 1) * 128] for h in hs], axis=1)
                    u = mxu_dot([weave.tie_m(xp[kb // 2])], w, kb % 2)
                    a = u if a is None else a + u
                    yield 8 * len(hs), u[:, 0:128]
                for i, t in enumerate(tiles(a)):
                    t = t - m * csq[:, hs[i] * 128:(hs[i] + 1) * 128]
                    q[g] = jnp.where(row == c0 + i, t, q[g]) if g in q else t

        def scores(g):
            s = [None] * 8
            for hf in range(2):
                for j, h in enumerate(groups[g]):
                    u = mxu_dot([weave.tie_m(pack(jnp.where(row == j, q[g], 0.0)))], k_half(h, hf))
                    for i, t in enumerate(tiles(u)):
                        accum(s, hf * 4 + i, t)
                    yield 32, u[:, 0:128]
            mx = lane_max(tree(jnp.maximum, s))
            e = [jnp.exp2((t - mx) * c) for t in s]
            p[g] = ([pack(e[i], e[i + 4]) for i in range(4)], 1.0 / lane_sum(tree(jnp.add, e)))

        def context(g):
            pk, rl = p[g]
            out = None
            for j, h in enumerate(groups[g]):
                a = None
                for hf in range(2):
                    u = mxu_dot([weave.tie_m(pk[0])] + pk[1:], v_half(h, hf), hf)
                    a = u if a is None else a + u
                    yield 32, u
                out = a if out is None else jnp.where(row == j, a, out)
            o[g] = out * rl

        def output(g):
            for c0 in range(0, len(groups[g]), 4):
                hs = groups[g][c0:c0 + 4]
                lhs = [pack(jnp.where(row == c0 + i, o[g], 0.0)) for i in range(len(hs))]
                for nt in range(DT):
                    w = jnp.concatenate([wo[h * 64:(h + 1) * 64, nt * 128:(nt + 1) * 128] for h in hs], axis=0)
                    u = mxu_dot([weave.tie_m(lhs[0])] + lhs[1:], w)
                    accum(macc, nt, u)
                    yield 8 * len(hs), u

        for t in range(len(groups) + 3):
            for d, stage in enumerate((project, scores, context, output)):
                if 0 <= t - d < len(groups):
                    yield from stage(t - d)

    def vpu():
        qcol, ocol, s, e, rl, qa, oa, seen = {}, {}, {}, {}, {}, {}, {}, {}

        def fold_rows(vals):
            low = (row & 4) == 0
            vals = [jnp.where(low, vals[k], vals[k + 4]) + pltpu.roll(jnp.where(low, vals[k + 4], vals[k]), 4, 0)
                    for k in range(4)]
            for sh in (2, 1):
                low = (row & sh) == 0
                vals = [jnp.where(low, vals[k] + pltpu.roll(vals[k], 8 - sh, 0),
                                  vals[k + sh] + pltpu.roll(vals[k + sh], sh, 0)) for k in range(sh)]
            return vals[0]

        def project(i):
            h, blk, sub = vheads[i // 16], (i % 16) // JB, i % JB
            js = range(blk * JB, (blk + 1) * JB)
            for kb in range(DT):
                if kb * JB // DT == sub:
                    x0 = weave.tie_v(xc[kb])
                    for j in js:
                        t = wqtf[h, j * 8:(j + 1) * 8, kb * 128:(kb + 1) * 128] * x0
                        qa[j] = t if kb == 0 else qa[j] + t
                    yield JB, qa[j]
            if sub == JB - 1:
                for j in js:
                    qcol[i // 16 * 16 + j] = lane_sum(qa[j])

        def scores(i):
            h, j = vheads[i // 16], i % 16
            sa = s.setdefault(h, [None] * 8)
            qc = weave.tie_v(qcol.pop(i))
            if i - 2 in seen:
                qc = jnp.where(weave.always, qc, seen.pop(i - 2))
            for t in range(8):
                accum(sa, t, ktf[h, j * 8:(j + 1) * 8, t * 128:(t + 1) * 128] * qc)
            seen[i] = sa[0]
            if j == 15:
                sc = fold_rows(s.pop(h))
                mx = lane_max(jnp.broadcast_to(jnp.max(sc, axis=0, keepdims=True), sc.shape))
                e[h] = jnp.exp2((sc - mx) * c)
                rl[h] = 1.0 / lane_sum(row_sum(e[h]))
            yield 8, sa[7]

        def context(i):
            h, blk, sub = vheads[i // 16], (i % 16) // JB, i % JB
            js = range(blk * JB, (blk + 1) * JB)
            for t in range(8):
                if t * JB // 8 == sub:
                    e0 = weave.tie_v(jnp.broadcast_to(e[h][t:t + 1, :], (8, DH)))
                    for j in js:
                        u = vtf[h, j * 8:(j + 1) * 8, t * 128:(t + 1) * 128] * e0
                        oa[j] = u if t == 0 else oa[j] + u
                    yield JB, oa[j]
            if sub == JB - 1:
                for j in js:
                    ocol[i // 16 * 16 + j] = lane_sum(oa[j]) * rl[h]

        def output(i):
            h, j = vheads[i // 16], i % 16
            oc = weave.tie_v(ocol.pop(i))
            for nt in range(DT):
                accum(vacc, nt, wof[h, j * 8:(j + 1) * 8, nt * 128:(nt + 1) * 128] * oc)
            yield 5, vacc[DT - 1]

        n = len(vheads) * 16
        stages = ((project, 0), (scores, 12), (context, 38), (output, 48))
        for step in range(n + stages[-1][1]):
            for stage, delay in stages:
                if 0 <= step - delay < n:
                    yield from stage(step - delay)

    weave.run(mxu(), sum(len(g) for g in groups) * 208, vpu(), len(vheads) * 416)
    return [xt[nt] + row_sum(macc[nt] + vacc[nt]) for nt in range(DT)]


def build_kernel(vpu_heads=(4, 3, 3, 3), mxu_groups=(3, 8, 8), fm=9, cuts=(0, 6, 8)):
    VG = max(vpu_heads)
    vheads = [g * VG + j for g in range(NG) for j in range(vpu_heads[g])]
    mheads = [g * G + j for g in range(NG) for j in range(vpu_heads[g], G)]
    groups = [mheads[sum(mxu_groups[:i]):sum(mxu_groups[:i + 1])] for i in range(len(mxu_groups))]
    FV = F - fm * 128
    LAST = NPAGE - 1
    FEED = (0, 5, 11, 13, 2 * NS)
    LAST_SLOTS = [(LAST - 1, i) for i in (9, 10, 13, 14, 15)] + [(LAST, i) for i in (5, 6, 7)]

    def kernel(x_hbm, k_hbm, v_hbm, wq_hbm, wo_hbm, w1t_hbm, b1_hbm, w2_hbm, b2_hbm, o_ref,
               kbuf, vbuf, kt, ktf, vtf,
               wq_raw, wo_raw, w1t_raw, w2_raw, x_raw, b1_raw, b2_raw,
               wq, wo, w1, w2, wqtf, wof, w1tf, w2f, csq, cs1, b1, b2, b1col,
               xin, xs, accs, ps, rls, res, zero, ksem, vsem, wsem, lsem):
        k32, v32 = kbuf.bitcast(u32), vbuf.bitcast(u32)

        def piece(src, buf, sem, t, hh, n, queue):
            r, size = sum(PIECE_ROWS[:n]), PIECE_ROWS[n]
            pltpu.make_async_copy(
                src.at[t // NG, (t % NG) * G + hh, pl.ds(SK - W + r, size), :],
                buf.at[t % buf.shape[0], hh, pl.ds(r, size), :], sem).start(priority=queue)

        def stripe(is_v, t, n):
            src, buf, sem = ((k_hbm, kbuf, ksem), (v_hbm, vbuf, vsem))[is_v]
            for i, hh in enumerate(HEAD_ORDER):
                piece(src, buf, sem.at[t % buf.shape[0]], t, hh, n, i % 2)

        def last_stripe(i):
            order = [(h + k * (G // 2), n) for h in range(G // 2) for n in range(NS) for k in range(2)]
            for hh, n in order[i * G:(i + 1) * G]:
                part = sum(hh >= c for c in cuts[1:-1])
                piece(v_hbm, vbuf, lsem.at[part], LAST, hh, n, hh // (G // 2))

        def slot(t, i):
            is_v, n = divmod(i, NS)
            for j, (tt, ii) in enumerate(LAST_SLOTS):
                if ii == i:
                    pl.when(t == tt)(lambda: last_stripe(j))
            swapped = LAST - 1 - is_v
            pl.when(t < swapped)(lambda: stripe(is_v, t + 1, n))
            pl.when(t == swapped)(lambda: stripe(1 - is_v, LAST - 1 + is_v, n))

        class Feed:
            def __init__(self, t, part, calls):
                self.t, self.lo, self.n, self.calls, self.k = t, FEED[part], FEED[part + 1] - FEED[part], calls, 0

            def __call__(self):
                a, e = (self.lo - (-self.n * k // self.calls) for k in (self.k, self.k + 1))
                self.k += 1
                for i in range(a, e):
                    slot(self.t, i)

        def wait(ref, sem):
            pltpu.make_async_copy(ref, ref, sem).wait()

        def fetch_wq(i):
            c = 0
            for n in (12 * 128, 10 * 128, 10 * 128):
                for k, h in enumerate(HEAD_ORDER):
                    at = (pl.ds(pl.multiple_of((h * 10 + i) * 8, 8), 8), pl.ds(c, n))
                    pltpu.make_async_copy(wq_hbm.at[at], wq_raw.at[at], wsem.at[0]).start(priority=k % 2)
                c += n

        def fetch_wo(i):
            for k, h in enumerate(HEAD_ORDER):
                at = pl.ds(pl.multiple_of(h * 512 + i * 16, 16), 16)
                pltpu.make_async_copy(wo_hbm.at[at, :], wo_raw.at[at, :], wsem.at[1]).start(priority=k % 2)

        def fetch_rows(src, dst, sem, i):
            for r in (0, 16):
                for q in range(2):
                    at = pl.ds(pl.multiple_of(i * 32 + r + q * (F // 2), 16), 16)
                    pltpu.make_async_copy(src.at[at, :], dst.at[at, :], sem).start(priority=q)

        def prep_wq(g):
            c = pl.ds(pl.multiple_of(g * G * DH, G * DH), G * DH)
            blk = wq_raw[:, c]
            wq[:, c] = pltpu.bitcast(blk, u32)
            csq[:, c] = jnp.dot(jnp.ones((16, D), bf16), blk, preferred_element_type=f32)[0:8]
            for j in range(VG):
                wqtf[g * VG + j] = blk[:, j * DH:(j + 1) * DH].T.astype(f32)

        def prep_wo(g):
            blk = wo_raw[pl.ds(pl.multiple_of(g * G * DH, G * DH), G * DH), :]
            wo[pl.ds(pl.multiple_of(g * G * 64, G * 64), G * 64), :] = pltpu.bitcast(blk, u32)
            for j in range(VG):
                wof[g * VG + j] = blk[j * DH:(j + 1) * DH].astype(f32)

        def prep_mlp(i):
            n = FP // 2
            r = pl.ds(pl.multiple_of(i * n, 128), n)
            blk = w1t_raw[r, :].T
            w1[:, r] = pltpu.bitcast(blk, u32)
            cs1[:, r] = jnp.dot(jnp.ones((16, D), bf16), blk, preferred_element_type=f32)[0:8]
            w2[pl.ds(pl.multiple_of(i * (n // 2), 64), n // 2), :] = pltpu.bitcast(w2_raw[r, :], u32)

        def prep_rest():
            b1v = jnp.concatenate([b1_raw[...].astype(f32)[None, :], jnp.zeros((1, FP - F), f32)], axis=1)
            b1[...] = jnp.broadcast_to(b1v, (8, FP))
            b2[...] = jnp.broadcast_to(b2_raw[...].astype(f32)[None, :], (8, D))

            def rows(i):
                r = pl.multiple_of(i * 64, 64)
                w1tf[pl.ds(r, 64), :] = w1t_raw[pl.ds(fm * 128 + r, 64), :].astype(f32)
                w2f[pl.ds(r, 64), :] = w2_raw[pl.ds(fm * 128 + r, 64), :].astype(f32)
            loop(FV // 64, rows)
            for c in range(fm, FP // 128):
                n = min(128, F - c * 128)
                t = jnp.broadcast_to(b1v[:, c * 128:(c + 1) * 128], (128, 128)).T
                b1col[(c - fm) * 128:(c - fm) * 128 + n, :] = t[0:n]

        def prep_late(t):
            @pl.when(t == 0)
            def _():
                wait(w1t_raw.at[pl.ds(0, F), :], wsem.at[2])
                wait(w2_raw.at[pl.ds(0, F), :], wsem.at[3])
                w1t_raw[F:FP, :] = jnp.zeros((FP - F, D), bf16)
                w2_raw[F:FP, :] = jnp.zeros((FP - F, D), bf16)
            pl.when(t < 2)(lambda: prep_mlp(t))
            pl.when(t == 2)(prep_rest)

        loop(10, fetch_wq)
        small = [pltpu.make_async_copy(x_hbm, x_raw, wsem.at[4]),
                 pltpu.make_async_copy(b1_hbm, b1_raw, wsem.at[5]),
                 pltpu.make_async_copy(b2_hbm, b2_raw, wsem.at[6])]
        for cp in small:
            cp.start()
        loop(32, fetch_wo)
        loop(F // 64, lambda i: fetch_rows(w1t_hbm, w1t_raw, wsem.at[2], i))
        wait(wq_raw, wsem.at[0])
        loop(NG, prep_wq)
        loop(F // 64, lambda i: fetch_rows(w2_hbm, w2_raw, wsem.at[3], i))
        wait(wo_raw, wsem.at[1])
        loop(NG, prep_wo)
        for is_v in range(2):
            for n in range(NS):
                stripe(is_v, 0, n)
        for cp in small:
            cp.wait()

        row = lax.broadcasted_iota(jnp.int32, (8, DH), 0)
        rowd = lax.broadcasted_iota(jnp.int32, (8, D), 0)
        xin[...] = x_raw[...].astype(f32)
        res[...] = jnp.zeros((8, D), f32)
        zero[...] = jnp.zeros((8, 128), jnp.int32)

        def start_layer(layer, x):
            xs[layer] = x
            accs[layer] = jnp.zeros((8, D), f32)

        def x_row(b):
            return jnp.broadcast_to(jnp.sum(jnp.where(rowd == b, xin[...], 0.0), axis=0, keepdims=True), (8, D))

        start_layer(0, x_row(0))

        def only_row(v, j):
            return unpack(pack(jnp.where(row == j, v, 0.0)))

        def queries(layer, g):
            c = pl.ds(pl.multiple_of(g * G * DH, G * DH), G * DH)
            x = xs[layer]
            m, var = moments(tiles(x))
            q = jnp.dot(jnp.concatenate([x, x], axis=0).astype(bf16), unpack(wq[:, c]),
                        preferred_element_type=f32)[0:8]
            return [t - m * cs for t, cs in zip(tiles(q), tiles(csq[:, c]))], lax.rsqrt(var + EPS) * SCALE

        def softmax(q, c, t, feed):
            s = None
            for j in range(G):
                feed()
                u = jnp.dot(only_row(q[j], j), unpack(kt[t % NV, j]), preferred_element_type=f32)[0:8]
                s = u if s is None else s + u
            s = tiles(s)
            mx = lane_max(tree(jnp.maximum, s))
            e = [jnp.exp2((u - mx) * c) for u in s]
            p = jnp.concatenate(e, axis=1)
            return jnp.concatenate([p, p], axis=0).astype(bf16), 1.0 / lane_sum(tree(jnp.add, e))

        def context(p, rl, t, js, feed=None):
            o = []
            for j in js:
                if feed:
                    feed()
                u = jnp.dot(p, unpack(v32[t % NV, j]), preferred_element_type=f32)[0:8]
                o.append(only_row(u * rl, j))
            r = ((t % NG) * G + js[0]) * 64
            r = r if isinstance(t, int) else pl.multiple_of(r, 64)
            return jnp.dot(jnp.concatenate(o, axis=1), unpack(wo[pl.ds(r, len(js) * 64), :]),
                           preferred_element_type=f32)[0:8]

        def transpose_v(t, js):
            for j in js:
                vtf[(t % NG) * VG + j] = unpack(v32[t % NV, j]).T.astype(f32)

        def after_attention(layer):
            return jnp.concatenate([a + row_sum(c) for a, c in zip(tiles(xs[layer]), tiles(accs[layer]))], axis=1)

        mlp_refs = (w1, w2, cs1, b1, b2, w1tf, w2f, b1col)

        def step(t):
            g = t % NG

            lo = jnp.where(t > LAST - 2, t + 1, t)
            hi = jnp.where(t < NG, t, jnp.minimum(jnp.where(t >= LAST - 2, t + 2, t + 1), NPAGE))

            def second_layer(u, carry):
                feed = Feed(jnp.where(u == lo, t, NPAGE), 0, 2 * G + 1)
                feed()
                p, rl = softmax(*queries(1, u % NG), u - NG, feed)
                accs[1] += context(p, rl, u - NG, range(G), feed)
                return carry
            lax.fori_loop(lo, hi, second_layer, 0)

            @pl.when(t < NG)
            def _():
                Feed(t, 0, 1)()
                prep_late(t)

            feed = Feed(t, 1, 2 * G + 1)
            wait(kbuf.at[t % NK], ksem.at[t % NK])
            feed()
            q, c = queries(0, g)
            for j in range(G):
                feed()
                kj = unpack(k32[t % NK, j]).T
                kt[t % NV, j] = pltpu.bitcast(kj, u32)
                if j < VG:
                    ktf[g * VG + j] = kj.astype(f32)
            ps[t % 2], rls[t % 2] = softmax(q, c, t, feed)

            tc = jnp.minimum(t, LAST - 1)

            @pl.when(t != LAST - 1)
            def _():
                wait(vbuf.at[tc % NV], vsem.at[tc % NV])
                transpose_v(tc, range(VG))
                accs[0] += context(ps[tc % 2], rls[tc % 2], tc, range(G), Feed(t, 2, G))

            first = (g == NG - 1) & (t < LAST)
            second = ((g == 0) & (t >= 2 * NG)) | (t == LAST - 1)

            @pl.when((first & (t >= NG)) | (t == LAST - 1))
            def _():
                xs[2] = after_attention(1)

            @pl.when(first)
            def _():
                xs[0] = after_attention(0)

            @pl.when(first | second)
            def _():
                x = mlp(tiles(xs[jnp.where(first, 0, 2)]), mlp_refs, FP // 128, Weave(None, FP, FP), 1,
                        Feed(t, 3, 4))
                x = jnp.concatenate(x, axis=1)

                @pl.when(first)
                def _():
                    start_layer(1, x)
                    start_layer(0, x_row(t // NG + 1))

                @pl.when(second)
                def _():
                    res[...] = jnp.where(rowd == (t + 2) // NG - 2, x, res[...])

            @pl.when(jnp.logical_not(first | second) & (t < LAST))
            def _():
                Feed(t, 3, 1)()

        loop(NPAGE, step)

        p, rl = ps[LAST % 2], rls[LAST % 2]
        acc = accs[0]
        for i, (lo, hi) in enumerate(zip(cuts[:-1], cuts[1:])):
            wait(vbuf.at[LAST % NV, pl.ds(lo, hi - lo)], lsem.at[i])
            transpose_v(LAST, range(lo, min(hi, vpu_heads[-1])))
            acc = acc + context(p, rl, LAST, range(lo, hi))
        xt = [a + row_sum(c) for a, c in zip(tiles(xs[0]), tiles(acc))]
        always = zero[...] == 0

        def k_half(h, hf):
            return kt[(NPAGE - NG + h // G) % NV, h % G, :, hf * 512:(hf + 1) * 512]

        def v_half(h, hf):
            return v32[(NPAGE - NG + h // G) % NV, h % G, hf * 256:(hf + 1) * 256, :]

        xt = mlp(xt, mlp_refs, fm, Weave(always, 4, 5, 0.1), 2)
        xt = attention(xt, (k_half, v_half, wq, wo, csq, ktf, vtf, wqtf, wof), vheads, groups, Weave(always, 4, 4))
        xt = mlp(xt, mlp_refs, fm, Weave(always, 4, 5, 0.1), 2)
        o_ref[...] = jnp.where(rowd == B - 1, jnp.concatenate(xt, axis=1), res[...]).astype(o_ref.dtype)

    V = pltpu.VMEM
    scratch = [
        V((NK, G, W, DH), bf16), V((NV, G, W, DH), bf16), V((NV, G, DH // 2, W), u32),
        V((NG * VG, DH, W), f32), V((NG * VG, DH, W), f32),
        V((D, H * DH), bf16), V((H * DH, D), bf16), V((FP, D), bf16), V((FP, D), bf16),
        V((B, D), bf16), V((F,), bf16), V((D,), bf16),
        V((D // 2, H * DH), u32), V((H * DH // 2, D), u32), V((D // 2, FP), u32), V((FP // 2, D), u32),
        V((NG * VG, DH, D), f32), V((NG * VG, DH, D), f32), V((FV, D), f32), V((FV, D), f32),
        V((8, H * DH), f32), V((8, FP), f32), V((8, FP), f32), V((8, D), f32), V((FV, 128), f32),
        V((8, D), f32), V((3, 8, D), f32), V((2, 8, D), f32), V((2, 16, W), bf16), V((2, 8, DH), f32),
        V((8, D), f32), V((8, 128), jnp.int32),
        pltpu.SemaphoreType.DMA((NK,)), pltpu.SemaphoreType.DMA((NV,)),
        pltpu.SemaphoreType.DMA((7,)), pltpu.SemaphoreType.DMA((len(cuts) - 1,)),
    ]

    return kernel, scratch


@jax.jit
def pallas_interleave_layers__sliding_block_cached__mixer_channel_mlp__decode_kernel(
    A_x: jax.Array,
    A_k_cache: jax.Array,
    A_v_cache: jax.Array,
    A_wq: jax.Array,
    A_wo: jax.Array,
    B_x: jax.Array,
    B_w1: jax.Array,
    B_b1: jax.Array,
    B_w2: jax.Array,
    B_b2: jax.Array,
):
    del B_x
    kernel, scratch = build_kernel()
    out = pl.pallas_call(
        kernel,
        in_specs=[pl.BlockSpec(memory_space=pltpu.HBM)] * 9,
        out_specs=pl.BlockSpec(memory_space=pltpu.VMEM),
        out_shape=jax.ShapeDtypeStruct((B, D), A_x.dtype),
        scratch_shapes=scratch,
        compiler_params=pltpu.CompilerParams(vmem_limit_bytes=124 * 1024 * 1024, disable_bounds_checks=True),
    )(A_x.reshape(B, D), A_k_cache, A_v_cache, A_wq, A_wo, B_w1.T, B_b1, B_w2, B_b2)
    return out.reshape(B, 1, D)
```

```python
import jax
import jax.numpy as jnp
from jax import lax
from jax.experimental import pallas as pl
from jax.experimental.pallas import tpu as pltpu

B, D, H, DH, SK, F = 8, 640, 32, 128, 4096, 1728
W = min(4096, max(256, SK // 4))
FP = 1792
DT = D // 128
G = 8
NG = H // G
NPAGE = B * NG
NK, NV = 4, 8
EPS = 1e-5
SCALE = DH ** -0.5 * 1.4426950408889634

PIECE_ROWS = (64, 96) * 6 + (64,)
NS = len(PIECE_ROWS)
REGIONS = (0, 4, 1, 5, 2, 6, 3, 7)

f32, bf16, u32 = jnp.float32, jnp.bfloat16, jnp.uint32


def tiles(v):
    return [v[:, i * 128:(i + 1) * 128] for i in range(v.shape[1] // 128)]


def tree(op, xs):
    xs = list(xs)
    while len(xs) > 1:
        xs = [op(*xs[i:i + 2]) if i + 1 < len(xs) else xs[i] for i in range(0, len(xs), 2)]
    return xs[0]


def lane_sum(v):
    return jnp.broadcast_to(jnp.sum(v, axis=1, keepdims=True), v.shape)


def lane_max(v):
    return jnp.broadcast_to(jnp.max(v, axis=1, keepdims=True), v.shape)


def row_sum(v):
    return jnp.broadcast_to(jnp.sum(v, axis=0, keepdims=True), v.shape)


def accum(acc, i, val):
    acc[i] = val if acc[i] is None else acc[i] + val


def pack(a, b=None):
    return pltpu.bitcast(jnp.concatenate([a, a if b is None else b], axis=0).astype(bf16), u32)


def unpack(w):
    return pltpu.bitcast(w, bf16)


def mxu_dot(lhs, w, half=0):
    lhs = jnp.concatenate([unpack(t) for t in lhs], axis=1)
    return jnp.dot(lhs, unpack(w), preferred_element_type=f32)[half * 8:half * 8 + 8]


def moments(xt):
    m = lane_sum(tree(jnp.add, xt)) * (1.0 / D)
    sq = lane_sum(tree(jnp.add, [t * t for t in xt])) * (1.0 / D)
    return m, jnp.maximum(sq - m * m, 0.0)


def gelu(x):
    c = 0.7978845608028654
    hx = 0.5 * x
    return hx + hx * jnp.tanh(x * (c + (c * 0.044715) * (x * x)))


def loop(n, body):
    lax.fori_loop(0, n, lambda i, c: (body(i), c)[1], 0)


class Weave:
    def __init__(self, always, lag_m, lag_v, lead=0.0):
        self.always, self.lag_m, self.lag_v, self.lead = always, lag_m, lag_v, lead
        self.vres, self.mres, self.fresh = [], [], False

    def tie_m(self, lhs):
        k = len(self.mres) - self.lag_m
        if k < 0 or self.vres[k] is None:
            return lhs
        return jnp.where(self.always, lhs, pltpu.bitcast(self.vres[k], u32))

    def tie_v(self, val):
        k = len(self.mres) - self.lag_v
        if k < 0 or not self.fresh:
            return val
        self.fresh = False
        return jnp.where(self.always, val, self.mres[k])

    def run(self, mxu, mxu_work, vpu, vpu_work):
        md = vd = 0
        last = None
        mxu_live, vpu_live = True, vpu_work > 0
        while mxu_live or vpu_live:
            if mxu_live and (not vpu_live or md / mxu_work <= -self.lead + (1 + self.lead) * vd / vpu_work):
                item = next(mxu, None)
                mxu_live = item is not None
                if mxu_live:
                    md += item[0]
                    self.vres.append(last)
                    self.mres.append(item[1])
                    self.fresh = True
            else:
                item = next(vpu, None)
                vpu_live = item is not None
                if vpu_live:
                    vd += item[0]
                    last = item[1]


JB = 4


def mlp(xt, refs, fm, weave, depth, feed=None):
    w1, w2, cs1, b1, b2, w1tf, w2f, b1col = refs
    m, var = moments(xt)
    r1 = lax.rsqrt(var + EPS)
    r = r1 * lax.rsqrt(var * r1 * r1 + EPS)
    xp = [pack(xt[i], xt[min(i + 1, DT - 1)]) for i in range(0, DT, 2)]
    xc = [t - m for t in xt]
    macc, vacc = [None] * DT, [None] * DT
    chunks = [(c, min(4, fm - c)) for c in range(0, fm, 4)]
    nj = max(F - fm * 128, 0) // 8

    def mxu():
        hs = {}

        def up(i):
            c0, n = chunks[i]
            a = None
            for kb in range(DT):
                u = mxu_dot([weave.tie_m(xp[kb // 2])], w1[kb * 64:(kb + 1) * 64, c0 * 128:(c0 + n) * 128], kb % 2)
                a = u if a is None else a + u
                yield 8 * n, u[:, 0:128]
            hs[i] = []
            for j, t in enumerate(tiles(a)):
                sl = slice((c0 + j) * 128, (c0 + j + 1) * 128)
                hs[i].append(pack(gelu((t - m * cs1[:, sl]) * r + b1[:, sl])))

        def down(i):
            c0, n = chunks[i]
            for nt in range(DT):
                u = mxu_dot([weave.tie_m(hs[i][0])] + hs[i][1:], w2[c0 * 64:(c0 + n) * 64, nt * 128:(nt + 1) * 128])
                accum(macc, nt, u)
                yield 8 * n, u

        for t in range(len(chunks) + depth):
            if t < len(chunks):
                if feed:
                    feed()
                yield from up(t)
            if t >= depth:
                yield from down(t - depth)

    def vpu():
        delay = 48
        col, part = {}, {}
        for step in range(nj + delay):
            if step < nj:
                blk, sub = divmod(step, JB)
                js = range(blk * JB, (blk + 1) * JB)
                for kb in range(DT):
                    if kb * JB // DT == sub:
                        x0 = weave.tie_v(xc[kb])
                        for j in js:
                            t = w1tf[j * 8:(j + 1) * 8, kb * 128:(kb + 1) * 128] * x0
                            part[j] = t if kb == 0 else part[j] + t
                        yield JB, part[j]
                if sub == JB - 1:
                    for j in js:
                        col[j] = lane_sum(part.pop(j))
            j = step - delay
            if j >= 0:
                h = weave.tie_v(gelu(col.pop(j) * r + b1col[j * 8:(j + 1) * 8, :]))
                for nt in range(DT):
                    accum(vacc, nt, w2f[j * 8:(j + 1) * 8, nt * 128:(nt + 1) * 128] * h)
                yield 5, vacc[DT - 1]

    weave.run(mxu(), fm * 80, vpu(), nj * 10)
    out = []
    for nt in range(DT):
        a = xt[nt] + b2[:, nt * 128:(nt + 1) * 128] + macc[nt]
        out.append(a if vacc[nt] is None else a + row_sum(vacc[nt]))
    return out


def attention(xt, refs, vheads, groups, weave):
    k_half, v_half, wq, wo, csq, ktf, vtf, wqtf, wof = refs
    row = lax.broadcasted_iota(jnp.int32, (8, DH), 0)
    m, var = moments(xt)
    c = lax.rsqrt(var + EPS) * SCALE
    xc = [t - m for t in xt]
    xp = [pack(xt[i], xt[min(i + 1, DT - 1)]) for i in range(0, DT, 2)]
    macc, vacc = [None] * DT, [None] * DT

    def mxu():
        q, p, o = {}, {}, {}

        def project(g):
            for c0 in range(0, len(groups[g]), 4):
                hs = groups[g][c0:c0 + 4]
                a = None
                for kb in range(DT):
                    w = jnp.concatenate([wq[kb * 64:(kb + 1) * 64, h * 128:(h + 1) * 128] for h in hs], axis=1)
                    u = mxu_dot([weave.tie_m(xp[kb // 2])], w, kb % 2)
                    a = u if a is None else a + u
                    yield 8 * len(hs), u[:, 0:128]
                for i, t in enumerate(tiles(a)):
                    t = t - m * csq[:, hs[i] * 128:(hs[i] + 1) * 128]
                    q[g] = jnp.where(row == c0 + i, t, q[g]) if g in q else t

        def scores(g):
            s = [None] * 8
            for hf in range(2):
                for j, h in enumerate(groups[g]):
                    u = mxu_dot([weave.tie_m(pack(jnp.where(row == j, q[g], 0.0)))], k_half(h, hf))
                    for i, t in enumerate(tiles(u)):
                        accum(s, hf * 4 + i, t)
                    yield 32, u[:, 0:128]
            mx = lane_max(tree(jnp.maximum, s))
            e = [jnp.exp2((t - mx) * c) for t in s]
            p[g] = ([pack(e[i], e[i + 4]) for i in range(4)], 1.0 / lane_sum(tree(jnp.add, e)))

        def context(g):
            pk, rl = p[g]
            out = None
            for j, h in enumerate(groups[g]):
                a = None
                for hf in range(2):
                    u = mxu_dot([weave.tie_m(pk[0])] + pk[1:], v_half(h, hf), hf)
                    a = u if a is None else a + u
                    yield 32, u
                out = a if out is None else jnp.where(row == j, a, out)
            o[g] = out * rl

        def output(g):
            for c0 in range(0, len(groups[g]), 4):
                hs = groups[g][c0:c0 + 4]
                lhs = [pack(jnp.where(row == c0 + i, o[g], 0.0)) for i in range(len(hs))]
                for nt in range(DT):
                    w = jnp.concatenate([wo[h * 64:(h + 1) * 64, nt * 128:(nt + 1) * 128] for h in hs], axis=0)
                    u = mxu_dot([weave.tie_m(lhs[0])] + lhs[1:], w)
                    accum(macc, nt, u)
                    yield 8 * len(hs), u

        for t in range(len(groups) + 3):
            for d, stage in enumerate((project, scores, context, output)):
                if 0 <= t - d < len(groups):
                    yield from stage(t - d)

    def vpu():
        qcol, ocol, s, e, rl, qa, oa, seen = {}, {}, {}, {}, {}, {}, {}, {}

        def fold_rows(vals):
            low = (row & 4) == 0
            vals = [jnp.where(low, vals[k], vals[k + 4]) + pltpu.roll(jnp.where(low, vals[k + 4], vals[k]), 4, 0)
                    for k in range(4)]
            for sh in (2, 1):
                low = (row & sh) == 0
                vals = [jnp.where(low, vals[k] + pltpu.roll(vals[k], 8 - sh, 0),
                                  vals[k + sh] + pltpu.roll(vals[k + sh], sh, 0)) for k in range(sh)]
            return vals[0]

        def project(i):
            h, blk, sub = vheads[i // 16], (i % 16) // JB, i % JB
            js = range(blk * JB, (blk + 1) * JB)
            for kb in range(DT):
                if kb * JB // DT == sub:
                    x0 = weave.tie_v(xc[kb])
                    for j in js:
                        t = wqtf[h, j * 8:(j + 1) * 8, kb * 128:(kb + 1) * 128] * x0
                        qa[j] = t if kb == 0 else qa[j] + t
                    yield JB, qa[j]
            if sub == JB - 1:
                for j in js:
                    qcol[i // 16 * 16 + j] = lane_sum(qa[j])

        def scores(i):
            h, j = vheads[i // 16], i % 16
            sa = s.setdefault(h, [None] * 8)
            qc = weave.tie_v(qcol.pop(i))
            if i - 2 in seen:
                qc = jnp.where(weave.always, qc, seen.pop(i - 2))
            for t in range(8):
                accum(sa, t, ktf[h, j * 8:(j + 1) * 8, t * 128:(t + 1) * 128] * qc)
            seen[i] = sa[0]
            if j == 15:
                sc = fold_rows(s.pop(h))
                mx = lane_max(jnp.broadcast_to(jnp.max(sc, axis=0, keepdims=True), sc.shape))
                e[h] = jnp.exp2((sc - mx) * c)
                rl[h] = 1.0 / lane_sum(row_sum(e[h]))
            yield 8, sa[7]

        def context(i):
            h, blk, sub = vheads[i // 16], (i % 16) // JB, i % JB
            js = range(blk * JB, (blk + 1) * JB)
            for t in range(8):
                if t * JB // 8 == sub:
                    e0 = weave.tie_v(jnp.broadcast_to(e[h][t:t + 1, :], (8, DH)))
                    for j in js:
                        u = vtf[h, j * 8:(j + 1) * 8, t * 128:(t + 1) * 128] * e0
                        oa[j] = u if t == 0 else oa[j] + u
                    yield JB, oa[j]
            if sub == JB - 1:
                for j in js:
                    ocol[i // 16 * 16 + j] = lane_sum(oa[j]) * rl[h]

        def output(i):
            h, j = vheads[i // 16], i % 16
            oc = weave.tie_v(ocol.pop(i))
            for nt in range(DT):
                accum(vacc, nt, wof[h, j * 8:(j + 1) * 8, nt * 128:(nt + 1) * 128] * oc)
            yield 5, vacc[DT - 1]

        n = len(vheads) * 16
        stages = ((project, 0), (scores, 12), (context, 38), (output, 48))
        for step in range(n + stages[-1][1]):
            for stage, delay in stages:
                if 0 <= step - delay < n:
                    yield from stage(step - delay)

    weave.run(mxu(), sum(len(g) for g in groups) * 208, vpu(), len(vheads) * 416)
    return [xt[nt] + row_sum(macc[nt] + vacc[nt]) for nt in range(DT)]


def build_kernel(vpu_heads=(4, 3, 3, 3), mxu_groups=(3, 8, 8), fm=9, cuts=(0, 6, 8), horder='04376215', behind=5, last_at=((21, 26), (9, 17)), feed_at=(9, 18, 21)):
    VG = max(vpu_heads)
    vheads = [g * VG + j for g in range(NG) for j in range(vpu_heads[g])]
    mheads = [g * G + j for g in range(NG) for j in range(vpu_heads[g], G)]
    groups = [mheads[sum(mxu_groups[:i]):sum(mxu_groups[:i + 1])] for i in range(len(mxu_groups))]
    FV = F - fm * 128
    LAST = NPAGE - 1
    FEED = (0, *feed_at, 2 * NS)

    LAST_SLOTS = [(LAST - 1 + k, i) for k, at in enumerate(last_at) for i in range(*at)]
    assert len(LAST_SLOTS) == NS and NS + behind <= FEED[2]

    def kernel(x_hbm, k_hbm, v_hbm, wq_hbm, wo_hbm, w1t_hbm, b1_hbm, w2_hbm, b2_hbm, o_ref,
               kbuf, vbuf, kt, ktf, vtf,
               wq_raw, wo_raw, w1t_raw, w2_raw, x_raw, b1_raw, b2_raw,
               wq, wo, w1, w2, wqtf, wof, w1tf, w2f, csq, cs1, b1, b2, b1col,
               xin, xs, accs, ps, rls, res, zero, ksem, vsem, wsem, lsem):
        k32, v32 = kbuf.bitcast(u32), vbuf.bitcast(u32)

        def piece(src, buf, sem, t, hh, n, queue):
            r, size = sum(PIECE_ROWS[:n]), PIECE_ROWS[n]
            pltpu.make_async_copy(
                src.at[t // NG, (t % NG) * G + hh, pl.ds(SK - W + r, size), :],
                buf.at[t % buf.shape[0], hh, pl.ds(r, size), :], sem).start(priority=queue)

        def stripe(is_v, t, n):
            src, buf, sem = ((k_hbm, kbuf, ksem), (v_hbm, vbuf, vsem))[is_v]
            for i, hh in enumerate(horder):
                piece(src, buf, sem.at[t % buf.shape[0]], t, int(hh), n, i % 2)

        def last_stripe(i):
            order = [(h + k * (G // 2), n) for h in range(G // 2) for n in range(NS) for k in range(2)]
            for hh, n in order[i * G:(i + 1) * G]:
                part = sum(hh >= c for c in cuts[1:-1])
                piece(v_hbm, vbuf, lsem.at[part], LAST, hh, n, hh // (G // 2))

        def slot(t, i):
            for n, (tt, ii) in enumerate(LAST_SLOTS):
                if ii == i:
                    pl.when(t == tt)(lambda: last_stripe(n))
            wrap, i = divmod(i - behind, 2 * NS)
            is_v, n = divmod(i, NS)
            page = t + 1 + wrap
            swapped = LAST - is_v
            pl.when(page < swapped)(lambda: stripe(is_v, page, n))
            pl.when(page == swapped)(lambda: stripe(1 - is_v, LAST - 1 + is_v, n))

        class Feed:
            def __init__(self, t, part, calls):
                self.t, self.lo, self.n, self.calls, self.k = t, FEED[part], FEED[part + 1] - FEED[part], calls, 0

            def __call__(self):
                a, e = (self.lo - (-self.n * k // self.calls) for k in (self.k, self.k + 1))
                self.k += 1
                for i in range(a, e):
                    slot(self.t, i)

        def wait(ref, sem):
            pltpu.make_async_copy(ref, ref, sem).wait()

        def fetch_wq(i):
            c = 0
            for n in (12 * 128, 10 * 128, 10 * 128):
                for k, h in enumerate(REGIONS):
                    at = (pl.ds(pl.multiple_of((h * 10 + i) * 8, 8), 8), pl.ds(c, n))
                    pltpu.make_async_copy(wq_hbm.at[at], wq_raw.at[at], wsem.at[0]).start(priority=k % 2)
                c += n

        def fetch_wo(i):
            for k, h in enumerate(REGIONS):
                at = pl.ds(pl.multiple_of(h * 512 + i * 16, 16), 16)
                pltpu.make_async_copy(wo_hbm.at[at, :], wo_raw.at[at, :], wsem.at[1]).start(priority=k % 2)

        def fetch_rows(src, dst, sem, i):
            for r in (0, 16):
                for q in range(2):
                    at = pl.ds(pl.multiple_of(i * 32 + r + q * (F // 2), 16), 16)
                    pltpu.make_async_copy(src.at[at, :], dst.at[at, :], sem).start(priority=q)

        def prep_wq(g):
            c = pl.ds(pl.multiple_of(g * G * DH, G * DH), G * DH)
            blk = wq_raw[:, c]
            wq[:, c] = pltpu.bitcast(blk, u32)
            csq[:, c] = jnp.dot(jnp.ones((16, D), bf16), blk, preferred_element_type=f32)[0:8]
            for j in range(VG):
                wqtf[g * VG + j] = blk[:, j * DH:(j + 1) * DH].T.astype(f32)

        def prep_wo(g):
            blk = wo_raw[pl.ds(pl.multiple_of(g * G * DH, G * DH), G * DH), :]
            wo[pl.ds(pl.multiple_of(g * G * 64, G * 64), G * 64), :] = pltpu.bitcast(blk, u32)
            for j in range(VG):
                wof[g * VG + j] = blk[j * DH:(j + 1) * DH].astype(f32)

        def prep_mlp(i):
            n = FP // 2
            r = pl.ds(pl.multiple_of(i * n, 128), n)
            blk = w1t_raw[r, :].T
            w1[:, r] = pltpu.bitcast(blk, u32)
            cs1[:, r] = jnp.dot(jnp.ones((16, D), bf16), blk, preferred_element_type=f32)[0:8]
            w2[pl.ds(pl.multiple_of(i * (n // 2), 64), n // 2), :] = pltpu.bitcast(w2_raw[r, :], u32)

        def prep_rest():
            b1v = jnp.concatenate([b1_raw[...].astype(f32)[None, :], jnp.zeros((1, FP - F), f32)], axis=1)
            b1[...] = jnp.broadcast_to(b1v, (8, FP))
            b2[...] = jnp.broadcast_to(b2_raw[...].astype(f32)[None, :], (8, D))

            def rows(i):
                r = pl.multiple_of(i * 64, 64)
                w1tf[pl.ds(r, 64), :] = w1t_raw[pl.ds(fm * 128 + r, 64), :].astype(f32)
                w2f[pl.ds(r, 64), :] = w2_raw[pl.ds(fm * 128 + r, 64), :].astype(f32)
            loop(FV // 64, rows)
            for c in range(fm, FP // 128):
                n = min(128, F - c * 128)
                t = jnp.broadcast_to(b1v[:, c * 128:(c + 1) * 128], (128, 128)).T
                b1col[(c - fm) * 128:(c - fm) * 128 + n, :] = t[0:n]

        def prep_late(t):
            @pl.when(t == 0)
            def _():
                wait(w1t_raw.at[pl.ds(0, F), :], wsem.at[2])
                wait(w2_raw.at[pl.ds(0, F), :], wsem.at[3])
                w1t_raw[F:FP, :] = jnp.zeros((FP - F, D), bf16)
                w2_raw[F:FP, :] = jnp.zeros((FP - F, D), bf16)
            pl.when(t < 2)(lambda: prep_mlp(t))
            pl.when(t == 2)(prep_rest)

        loop(10, fetch_wq)
        small = [pltpu.make_async_copy(x_hbm, x_raw, wsem.at[4]),
                 pltpu.make_async_copy(b1_hbm, b1_raw, wsem.at[5]),
                 pltpu.make_async_copy(b2_hbm, b2_raw, wsem.at[6])]
        for cp in small:
            cp.start()
        loop(32, fetch_wo)
        loop(F // 64, lambda i: fetch_rows(w1t_hbm, w1t_raw, wsem.at[2], i))
        wait(wq_raw, wsem.at[0])
        loop(NG, prep_wq)
        loop(F // 64, lambda i: fetch_rows(w2_hbm, w2_raw, wsem.at[3], i))
        wait(wo_raw, wsem.at[1])
        loop(NG, prep_wo)
        for i in range(2 * NS - behind):
            stripe(i // NS, 0, i % NS)
        for cp in small:
            cp.wait()

        row = lax.broadcasted_iota(jnp.int32, (8, DH), 0)
        rowd = lax.broadcasted_iota(jnp.int32, (8, D), 0)
        xin[...] = x_raw[...].astype(f32)
        res[...] = jnp.zeros((8, D), f32)
        zero[...] = jnp.zeros((8, 128), jnp.int32)

        def start_layer(layer, x):
            xs[layer] = x
            accs[layer] = jnp.zeros((8, D), f32)

        def x_row(b):
            return jnp.broadcast_to(jnp.sum(jnp.where(rowd == b, xin[...], 0.0), axis=0, keepdims=True), (8, D))

        start_layer(0, x_row(0))

        def only_row(v, j):
            return unpack(pack(jnp.where(row == j, v, 0.0)))

        def queries(layer, g):
            c = pl.ds(pl.multiple_of(g * G * DH, G * DH), G * DH)
            x = xs[layer]
            m, var = moments(tiles(x))
            q = jnp.dot(jnp.concatenate([x, x], axis=0).astype(bf16), unpack(wq[:, c]),
                        preferred_element_type=f32)[0:8]
            return [t - m * cs for t, cs in zip(tiles(q), tiles(csq[:, c]))], lax.rsqrt(var + EPS) * SCALE

        def softmax(q, c, t, feed):
            s = None
            for j in range(G):
                feed()
                u = jnp.dot(only_row(q[j], j), unpack(kt[t % NV, j]), preferred_element_type=f32)[0:8]
                s = u if s is None else s + u
            s = tiles(s)
            mx = lane_max(tree(jnp.maximum, s))
            e = [jnp.exp2((u - mx) * c) for u in s]
            p = jnp.concatenate(e, axis=1)
            return jnp.concatenate([p, p], axis=0).astype(bf16), 1.0 / lane_sum(tree(jnp.add, e))

        def context(p, rl, t, js, feed=None):
            o = []
            for j in js:
                if feed:
                    feed()
                u = jnp.dot(p, unpack(v32[t % NV, j]), preferred_element_type=f32)[0:8]
                o.append(only_row(u * rl, j))
            r = ((t % NG) * G + js[0]) * 64
            r = r if isinstance(t, int) else pl.multiple_of(r, 64)
            return jnp.dot(jnp.concatenate(o, axis=1), unpack(wo[pl.ds(r, len(js) * 64), :]),
                           preferred_element_type=f32)[0:8]

        def transpose_v(t, js):
            for j in js:
                vtf[(t % NG) * VG + j] = unpack(v32[t % NV, j]).T.astype(f32)

        def after_attention(layer):
            return jnp.concatenate([a + row_sum(c) for a, c in zip(tiles(xs[layer]), tiles(accs[layer]))], axis=1)

        mlp_refs = (w1, w2, cs1, b1, b2, w1tf, w2f, b1col)

        def step(t):
            g = t % NG

            lo = jnp.where(t > LAST - 2, t + 1, t)
            hi = jnp.where(t < NG, t, jnp.minimum(jnp.where(t >= LAST - 2, t + 2, t + 1), NPAGE))

            def second_layer(u, carry):
                feed = Feed(jnp.where(u == lo, t, NPAGE), 0, 2 * G + 1)
                feed()
                p, rl = softmax(*queries(1, u % NG), u - NG, feed)
                accs[1] += context(p, rl, u - NG, range(G), feed)
                return carry
            lax.fori_loop(lo, hi, second_layer, 0)

            @pl.when(t < NG)
            def _():
                Feed(t, 0, 1)()
                prep_late(t)

            feed = Feed(t, 1, 2 * G + 1)
            wait(kbuf.at[t % NK], ksem.at[t % NK])
            feed()
            q, c = queries(0, g)
            for j in range(G):
                feed()
                kj = unpack(k32[t % NK, j]).T
                kt[t % NV, j] = pltpu.bitcast(kj, u32)
                if j < VG:
                    ktf[g * VG + j] = kj.astype(f32)
            ps[t % 2], rls[t % 2] = softmax(q, c, t, feed)

            tc = jnp.minimum(t, LAST - 1)

            @pl.when(t != LAST - 1)
            def _():
                wait(vbuf.at[tc % NV], vsem.at[tc % NV])
                transpose_v(tc, range(VG))
                accs[0] += context(ps[tc % 2], rls[tc % 2], tc, range(G), Feed(t, 2, G))

            first = (g == NG - 1) & (t < LAST)
            second = ((g == 0) & (t >= 2 * NG)) | (t == LAST - 1)

            @pl.when((first & (t >= NG)) | (t == LAST - 1))
            def _():
                xs[2] = after_attention(1)

            @pl.when(first)
            def _():
                xs[0] = after_attention(0)

            @pl.when(first | second)
            def _():
                x = mlp(tiles(xs[jnp.where(first, 0, 2)]), mlp_refs, FP // 128, Weave(None, FP, FP), 1,
                        Feed(t, 3, 4))
                x = jnp.concatenate(x, axis=1)

                @pl.when(first)
                def _():
                    start_layer(1, x)
                    start_layer(0, x_row(t // NG + 1))

                @pl.when(second)
                def _():
                    res[...] = jnp.where(rowd == (t + 2) // NG - 2, x, res[...])

            @pl.when(jnp.logical_not(first | second) & (t < LAST))
            def _():
                Feed(t, 3, 1)()

        loop(NPAGE, step)

        p, rl = ps[LAST % 2], rls[LAST % 2]
        acc = accs[0]
        for i, (lo, hi) in enumerate(zip(cuts[:-1], cuts[1:])):
            wait(vbuf.at[LAST % NV, pl.ds(lo, hi - lo)], lsem.at[i])
            transpose_v(LAST, range(lo, min(hi, vpu_heads[-1])))
            acc = acc + context(p, rl, LAST, range(lo, hi))
        xt = [a + row_sum(c) for a, c in zip(tiles(xs[0]), tiles(acc))]
        always = zero[...] == 0

        def k_half(h, hf):
            return kt[(NPAGE - NG + h // G) % NV, h % G, :, hf * 512:(hf + 1) * 512]

        def v_half(h, hf):
            return v32[(NPAGE - NG + h // G) % NV, h % G, hf * 256:(hf + 1) * 256, :]

        xt = mlp(xt, mlp_refs, fm, Weave(always, 4, 5, 0.1), 2)
        xt = attention(xt, (k_half, v_half, wq, wo, csq, ktf, vtf, wqtf, wof), vheads, groups, Weave(always, 4, 4))
        xt = mlp(xt, mlp_refs, fm, Weave(always, 4, 5, 0.1), 2)
        o_ref[...] = jnp.where(rowd == B - 1, jnp.concatenate(xt, axis=1), res[...]).astype(o_ref.dtype)

    V = pltpu.VMEM
    scratch = [
        V((NK, G, W, DH), bf16), V((NV, G, W, DH), bf16), V((NV, G, DH // 2, W), u32),
        V((NG * VG, DH, W), f32), V((NG * VG, DH, W), f32),
        V((D, H * DH), bf16), V((H * DH, D), bf16), V((FP, D), bf16), V((FP, D), bf16),
        V((B, D), bf16), V((F,), bf16), V((D,), bf16),
        V((D // 2, H * DH), u32), V((H * DH // 2, D), u32), V((D // 2, FP), u32), V((FP // 2, D), u32),
        V((NG * VG, DH, D), f32), V((NG * VG, DH, D), f32), V((FV, D), f32), V((FV, D), f32),
        V((8, H * DH), f32), V((8, FP), f32), V((8, FP), f32), V((8, D), f32), V((FV, 128), f32),
        V((8, D), f32), V((3, 8, D), f32), V((2, 8, D), f32), V((2, 16, W), bf16), V((2, 8, DH), f32),
        V((8, D), f32), V((8, 128), jnp.int32),
        pltpu.SemaphoreType.DMA((NK,)), pltpu.SemaphoreType.DMA((NV,)),
        pltpu.SemaphoreType.DMA((7,)), pltpu.SemaphoreType.DMA((len(cuts) - 1,)),
    ]

    return kernel, scratch


@jax.jit
def pallas_interleave_layers__sliding_block_cached__mixer_channel_mlp__decode_kernel(
    A_x: jax.Array,
    A_k_cache: jax.Array,
    A_v_cache: jax.Array,
    A_wq: jax.Array,
    A_wo: jax.Array,
    B_x: jax.Array,
    B_w1: jax.Array,
    B_b1: jax.Array,
    B_w2: jax.Array,
    B_b2: jax.Array,
):
    del B_x
    kernel, scratch = build_kernel()
    out = pl.pallas_call(
        kernel,
        in_specs=[pl.BlockSpec(memory_space=pltpu.HBM)] * 9,
        out_specs=pl.BlockSpec(memory_space=pltpu.VMEM),
        out_shape=jax.ShapeDtypeStruct((B, D), A_x.dtype),
        scratch_shapes=scratch,
        compiler_params=pltpu.CompilerParams(vmem_limit_bytes=124 * 1024 * 1024, disable_bounds_checks=True),
    )(A_x.reshape(B, D), A_k_cache, A_v_cache, A_wq, A_wo, B_w1.T, B_b1, B_w2, B_b2)
    return out.reshape(B, 1, D)
```

```python
import jax
import jax.numpy as jnp
from jax import lax
from jax.experimental import pallas as pl
from jax.experimental.pallas import tpu as pltpu

B, D, H, DH, SK, F = 8, 640, 32, 128, 4096, 1728
W = min(4096, max(256, SK // 4))
FP = 1792
DT = D // 128
G = 8
NG = H // G
NPAGE = B * NG
NK, NV = 4, 8
EPS = 1e-5
SCALE = DH ** -0.5 * 1.4426950408889634

PIECE_ROWS = (64, 96) * 6 + (64,)
NS = len(PIECE_ROWS)
REGIONS = (0, 4, 1, 5, 2, 6, 3, 7)

f32, bf16, u32 = jnp.float32, jnp.bfloat16, jnp.uint32


def tiles(v):
    return [v[:, i * 128:(i + 1) * 128] for i in range(v.shape[1] // 128)]


def tree(op, xs):
    xs = list(xs)
    while len(xs) > 1:
        xs = [op(*xs[i:i + 2]) if i + 1 < len(xs) else xs[i] for i in range(0, len(xs), 2)]
    return xs[0]


def lane_sum(v):
    return jnp.broadcast_to(jnp.sum(v, axis=1, keepdims=True), v.shape)


def lane_max(v):
    return jnp.broadcast_to(jnp.max(v, axis=1, keepdims=True), v.shape)


def row_sum(v):
    return jnp.broadcast_to(jnp.sum(v, axis=0, keepdims=True), v.shape)


def accum(acc, i, val):
    acc[i] = val if acc[i] is None else acc[i] + val


def pack(a, b=None):
    return pltpu.bitcast(jnp.concatenate([a, a if b is None else b], axis=0).astype(bf16), u32)


def unpack(w):
    return pltpu.bitcast(w, bf16)


def mxu_dot(lhs, w, half=0):
    lhs = jnp.concatenate([unpack(t) for t in lhs], axis=1)
    return jnp.dot(lhs, unpack(w), preferred_element_type=f32)[half * 8:half * 8 + 8]


def moments(xt):
    m = lane_sum(tree(jnp.add, xt)) * (1.0 / D)
    sq = lane_sum(tree(jnp.add, [t * t for t in xt])) * (1.0 / D)
    return m, jnp.maximum(sq - m * m, 0.0)


def gelu(x):
    c = 0.7978845608028654
    hx = 0.5 * x
    return hx + hx * jnp.tanh(x * (c + (c * 0.044715) * (x * x)))


def loop(n, body):
    lax.fori_loop(0, n, lambda i, c: (body(i), c)[1], 0)


class Weave:
    def __init__(self, always, lag_m, lag_v, lead=0.0):
        self.always, self.lag_m, self.lag_v, self.lead = always, lag_m, lag_v, lead
        self.vres, self.mres, self.fresh = [], [], False

    def tie_m(self, lhs):
        k = len(self.mres) - self.lag_m
        if k < 0 or self.vres[k] is None:
            return lhs
        return jnp.where(self.always, lhs, pltpu.bitcast(self.vres[k], u32))

    def tie_v(self, val):
        k = len(self.mres) - self.lag_v
        if k < 0 or not self.fresh:
            return val
        self.fresh = False
        return jnp.where(self.always, val, self.mres[k])

    def run(self, mxu, mxu_work, vpu, vpu_work):
        md = vd = 0
        last = None
        mxu_live, vpu_live = True, vpu_work > 0
        while mxu_live or vpu_live:
            if mxu_live and (not vpu_live or md / mxu_work <= -self.lead + (1 + self.lead) * vd / vpu_work):
                item = next(mxu, None)
                mxu_live = item is not None
                if mxu_live:
                    md += item[0]
                    self.vres.append(last)
                    self.mres.append(item[1])
                    self.fresh = True
            else:
                item = next(vpu, None)
                vpu_live = item is not None
                if vpu_live:
                    vd += item[0]
                    last = item[1]


JB = 4


def mlp(xt, refs, fm, weave, depth, feed=None, delay=48):
    w1, w2, cs1, b1, b2, w1tf, w2f, b1col = refs
    m, var = moments(xt)
    r1 = lax.rsqrt(var + EPS)
    r = r1 * lax.rsqrt(var * r1 * r1 + EPS)
    xp = [pack(xt[i], xt[min(i + 1, DT - 1)]) for i in range(0, DT, 2)]
    xc = [t - m for t in xt]
    macc, vacc = [None] * DT, [None] * DT
    chunks = [(c, min(4, fm - c)) for c in range(0, fm, 4)]
    nj = max(F - fm * 128, 0) // 8

    def mxu():
        hs = {}

        def up(i):
            c0, n = chunks[i]
            a = None
            for kb in range(DT):
                u = mxu_dot([weave.tie_m(xp[kb // 2])], w1[kb * 64:(kb + 1) * 64, c0 * 128:(c0 + n) * 128], kb % 2)
                a = u if a is None else a + u
                yield 8 * n, u[:, 0:128]
            hs[i] = []
            for j, t in enumerate(tiles(a)):
                sl = slice((c0 + j) * 128, (c0 + j + 1) * 128)
                hs[i].append(pack(gelu((t - m * cs1[:, sl]) * r + b1[:, sl])))

        def down(i):
            c0, n = chunks[i]
            for nt in range(DT):
                u = mxu_dot([weave.tie_m(hs[i][0])] + hs[i][1:], w2[c0 * 64:(c0 + n) * 64, nt * 128:(nt + 1) * 128])
                accum(macc, nt, u)
                yield 8 * n, u

        for t in range(len(chunks) + depth):
            if t < len(chunks):
                if feed:
                    feed()
                yield from up(t)
            if t >= depth:
                yield from down(t - depth)

    def vpu():
        col, part = {}, {}
        for step in range(nj + delay):
            if step < nj:
                blk, sub = divmod(step, JB)
                js = range(blk * JB, (blk + 1) * JB)
                for kb in range(DT):
                    if kb * JB // DT == sub:
                        x0 = weave.tie_v(xc[kb])
                        for j in js:
                            t = w1tf[j * 8:(j + 1) * 8, kb * 128:(kb + 1) * 128] * x0
                            part[j] = t if kb == 0 else part[j] + t
                        yield JB, part[j]
                if sub == JB - 1:
                    for j in js:
                        col[j] = lane_sum(part.pop(j))
            j = step - delay
            if j >= 0:
                h = weave.tie_v(gelu(col.pop(j) * r + b1col[j * 8:(j + 1) * 8, :]))
                for nt in range(DT):
                    accum(vacc, nt, w2f[j * 8:(j + 1) * 8, nt * 128:(nt + 1) * 128] * h)
                yield 5, vacc[DT - 1]

    weave.run(mxu(), fm * 80, vpu(), nj * 10)
    out = []
    for nt in range(DT):
        a = xt[nt] + b2[:, nt * 128:(nt + 1) * 128] + macc[nt]
        out.append(a if vacc[nt] is None else a + row_sum(vacc[nt]))
    return out


def attention(xt, refs, vheads, groups, weave, delays, order, back):
    k_half, v_half, wq, wo, csq, ktf, vtf, wqtf, wof = refs
    row = lax.broadcasted_iota(jnp.int32, (8, DH), 0)
    m, var = moments(xt)
    c = lax.rsqrt(var + EPS) * SCALE
    xc = [t - m for t in xt]
    xp = [pack(xt[i], xt[min(i + 1, DT - 1)]) for i in range(0, DT, 2)]
    macc, vacc = [None] * DT, [None] * DT

    def mxu():
        q, p, o = {}, {}, {}

        def project(g):
            for c0 in range(0, len(groups[g]), 4):
                hs = groups[g][c0:c0 + 4]
                a = None
                for kb in range(DT):
                    w = jnp.concatenate([wq[kb * 64:(kb + 1) * 64, h * 128:(h + 1) * 128] for h in hs], axis=1)
                    u = mxu_dot([weave.tie_m(xp[kb // 2])], w, kb % 2)
                    a = u if a is None else a + u
                    yield 8 * len(hs), u[:, 0:128]
                for i, t in enumerate(tiles(a)):
                    t = t - m * csq[:, hs[i] * 128:(hs[i] + 1) * 128]
                    q[g] = jnp.where(row == c0 + i, t, q[g]) if g in q else t

        def scores(g):
            s = [None] * 8
            for hf in range(2):
                for j, h in enumerate(groups[g]):
                    u = mxu_dot([weave.tie_m(pack(jnp.where(row == j, q[g], 0.0)))], k_half(h, hf))
                    for i, t in enumerate(tiles(u)):
                        accum(s, hf * 4 + i, t)
                    yield 32, u[:, 0:128]
            mx = lane_max(tree(jnp.maximum, s))
            e = [jnp.exp2((t - mx) * c) for t in s]
            p[g] = ([pack(e[i], e[i + 4]) for i in range(4)], 1.0 / lane_sum(tree(jnp.add, e)))

        def context(g):
            pk, rl = p[g]
            out = None
            for j, h in enumerate(groups[g]):
                a = None
                for hf in range(2):
                    u = mxu_dot([weave.tie_m(pk[0])] + pk[1:], v_half(h, hf), hf)
                    a = u if a is None else a + u
                    yield 32, u
                out = a if out is None else jnp.where(row == j, a, out)
            o[g] = out * rl

        def output(g):
            for c0 in range(0, len(groups[g]), 4):
                hs = groups[g][c0:c0 + 4]
                lhs = [pack(jnp.where(row == c0 + i, o[g], 0.0)) for i in range(len(hs))]
                for nt in range(DT):
                    w = jnp.concatenate([wo[h * 64:(h + 1) * 64, nt * 128:(nt + 1) * 128] for h in hs], axis=0)
                    u = mxu_dot([weave.tie_m(lhs[0])] + lhs[1:], w)
                    accum(macc, nt, u)
                    yield 8 * len(hs), u

        for t in range(len(groups) + 3):
            for d, stage in enumerate((project, scores, context, output)):
                if 0 <= t - d < len(groups):
                    yield from stage(t - d)

    def vpu():
        qcol, ocol, s, e, rl, qa, oa, seen = {}, {}, {}, {}, {}, {}, {}, {}

        def fold_rows(vals):
            low = (row & 4) == 0
            vals = [jnp.where(low, vals[k], vals[k + 4]) + pltpu.roll(jnp.where(low, vals[k + 4], vals[k]), 4, 0)
                    for k in range(4)]
            for sh in (2, 1):
                low = (row & sh) == 0
                vals = [jnp.where(low, vals[k] + pltpu.roll(vals[k], 8 - sh, 0),
                                  vals[k + sh] + pltpu.roll(vals[k + sh], sh, 0)) for k in range(sh)]
            return vals[0]

        def project(i):
            h, blk, sub = vheads[i // 16], (i % 16) // JB, i % JB
            js = range(blk * JB, (blk + 1) * JB)
            for kb in range(DT):
                if kb * JB // DT == sub:
                    x0 = weave.tie_v(xc[kb])
                    for j in js:
                        t = wqtf[h, j * 8:(j + 1) * 8, kb * 128:(kb + 1) * 128] * x0
                        qa[j] = t if kb == 0 else qa[j] + t
                    yield JB, qa[j]
            if sub == JB - 1:
                for j in js:
                    qcol[i // 16 * 16 + j] = lane_sum(qa[j])

        def scores(i):
            h, j = vheads[i // 16], i % 16
            sa = s.setdefault(h, [None] * 8)
            qc = weave.tie_v(qcol.pop(i))
            if i - back in seen:
                qc = jnp.where(weave.always, qc, seen.pop(i - back))
            for t in range(8):
                accum(sa, t, ktf[h, j * 8:(j + 1) * 8, t * 128:(t + 1) * 128] * qc)
            seen[i] = sa[0]
            if j == 15:
                sc = fold_rows(s.pop(h))
                mx = lane_max(jnp.broadcast_to(jnp.max(sc, axis=0, keepdims=True), sc.shape))
                e[h] = jnp.exp2((sc - mx) * c)
                rl[h] = 1.0 / lane_sum(row_sum(e[h]))
            yield 8, sa[7]

        def context(i):
            h, blk, sub = vheads[i // 16], (i % 16) // JB, i % JB
            js = range(blk * JB, (blk + 1) * JB)
            for t in range(8):
                if t * JB // 8 == sub:
                    e0 = weave.tie_v(jnp.broadcast_to(e[h][t:t + 1, :], (8, DH)))
                    for j in js:
                        u = vtf[h, j * 8:(j + 1) * 8, t * 128:(t + 1) * 128] * e0
                        oa[j] = u if t == 0 else oa[j] + u
                    yield JB, oa[j]
            if sub == JB - 1:
                for j in js:
                    ocol[i // 16 * 16 + j] = lane_sum(oa[j]) * rl[h]

        def output(i):
            h, j = vheads[i // 16], i % 16
            oc = weave.tie_v(ocol.pop(i))
            for nt in range(DT):
                accum(vacc, nt, wof[h, j * 8:(j + 1) * 8, nt * 128:(nt + 1) * 128] * oc)
            yield 5, vacc[DT - 1]

        n = len(vheads) * 16
        stages = list(zip((project, scores, context, output), delays))
        stages = [stages[int(k)] for k in order]
        for step in range(n + delays[-1]):
            for stage, delay in stages:
                if 0 <= step - delay < n:
                    yield from stage(step - delay)

    weave.run(mxu(), sum(len(g) for g in groups) * 208, vpu(), len(vheads) * 416)
    return [xt[nt] + row_sum(macc[nt] + vacc[nt]) for nt in range(DT)]


def build_kernel(vpu_heads=(4, 3, 3, 3), mxu_groups=(4, 8, 7), fm=9, cuts=(0, 6, 8), horder='04376215', behind=5, last_at=((23, 26), (9, 19)), feed_at=(9, 19, 21),
         m1=(99, 99, 0, 1, 32), m2=(3, 5, 0.1, 2, 48), lag=(3, 4, 0), delays=(0, 10, 36, 48), vorder='0123', back=2):
    VG = max(vpu_heads)
    vheads = [g * VG + j for g in range(NG) for j in range(vpu_heads[g])]
    mheads = [g * G + j for g in range(NG) for j in range(vpu_heads[g], G)]
    groups = [mheads[sum(mxu_groups[:i]):sum(mxu_groups[:i + 1])] for i in range(len(mxu_groups))]
    FV = F - fm * 128
    LAST = NPAGE - 1
    FEED = (0, *feed_at, 2 * NS)

    LAST_SLOTS = [(LAST - 1 + k, i) for k, at in enumerate(last_at) for i in range(*at)]
    assert len(LAST_SLOTS) == NS and NS + behind <= FEED[2]
    assert all(i >= FEED[3] if t < LAST else FEED[1] <= i < FEED[3] for t, i in LAST_SLOTS)

    def kernel(x_hbm, k_hbm, v_hbm, wq_hbm, wo_hbm, w1t_hbm, b1_hbm, w2_hbm, b2_hbm, o_ref,
               kbuf, vbuf, kt, ktf, vtf,
               wq_raw, wo_raw, w1t_raw, w2_raw, x_raw, b1_raw, b2_raw,
               wq, wo, w1, w2, wqtf, wof, w1tf, w2f, csq, cs1, b1, b2, b1col,
               xin, xs, accs, ps, rls, res, zero, ksem, vsem, wsem, lsem):
        k32, v32 = kbuf.bitcast(u32), vbuf.bitcast(u32)

        def piece(src, buf, sem, t, hh, n, queue):
            r, size = sum(PIECE_ROWS[:n]), PIECE_ROWS[n]
            pltpu.make_async_copy(
                src.at[t // NG, (t % NG) * G + hh, pl.ds(SK - W + r, size), :],
                buf.at[t % buf.shape[0], hh, pl.ds(r, size), :], sem).start(priority=queue)

        def stripe(is_v, t, n):
            src, buf, sem = ((k_hbm, kbuf, ksem), (v_hbm, vbuf, vsem))[is_v]
            for i, hh in enumerate(horder):
                piece(src, buf, sem.at[t % buf.shape[0]], t, int(hh), n, i % 2)

        def last_stripe(i):
            order = [(h + k * (G // 2), n) for h in range(G // 2) for n in range(NS) for k in range(2)]
            for hh, n in order[i * G:(i + 1) * G]:
                part = sum(hh >= c for c in cuts[1:-1])
                piece(v_hbm, vbuf, lsem.at[part], LAST, hh, n, hh // (G // 2))

        def slot(t, i):
            for n, (tt, ii) in enumerate(LAST_SLOTS):
                if ii == i:
                    pl.when(t == tt)(lambda: last_stripe(n))
            wrap, i = divmod(i - behind, 2 * NS)
            is_v, n = divmod(i, NS)
            page = t + 1 + wrap
            swapped = LAST - is_v
            pl.when(page < swapped)(lambda: stripe(is_v, page, n))
            pl.when(page == swapped)(lambda: stripe(1 - is_v, LAST - 1 + is_v, n))

        class Feed:
            def __init__(self, t, part, calls):
                self.t, self.lo, self.n, self.calls, self.k = t, FEED[part], FEED[part + 1] - FEED[part], calls, 0

            def __call__(self):
                a, e = (self.lo - (-self.n * k // self.calls) for k in (self.k, self.k + 1))
                self.k += 1
                for i in range(a, e):
                    slot(self.t, i)

        def wait(ref, sem):
            pltpu.make_async_copy(ref, ref, sem).wait()

        def fetch_wq(i):
            c = 0
            for n in (8 * 128, 12 * 128, 12 * 128):
                for k, h in enumerate(REGIONS):
                    at = (pl.ds(pl.multiple_of((h * 10 + i) * 8, 8), 8), pl.ds(c, n))
                    pltpu.make_async_copy(wq_hbm.at[at], wq_raw.at[at], wsem.at[0]).start(priority=k % 2)
                c += n

        def fetch_wo(i):
            for r, n in ((0, 8), (8, 24)):
                for k, h in enumerate(REGIONS):
                    at = pl.ds(pl.multiple_of(h * 512 + i * 32 + r, 8), n)
                    pltpu.make_async_copy(wo_hbm.at[at, :], wo_raw.at[at, :], wsem.at[1]).start(priority=k % 2)

        def fetch_rows(src, dst, sem, i):
            for r in (0, 16):
                for q in range(2):
                    at = pl.ds(pl.multiple_of(i * 32 + r + q * (F // 2), 16), 16)
                    pltpu.make_async_copy(src.at[at, :], dst.at[at, :], sem).start(priority=q)

        def prep_wq(g):
            c = pl.ds(pl.multiple_of(g * G * DH, G * DH), G * DH)
            blk = wq_raw[:, c]
            wq[:, c] = pltpu.bitcast(blk, u32)
            csq[:, c] = jnp.dot(jnp.ones((16, D), bf16), blk, preferred_element_type=f32)[0:8]
            for j in range(VG):
                wqtf[g * VG + j] = blk[:, j * DH:(j + 1) * DH].T.astype(f32)

        def prep_wo(g):
            blk = wo_raw[pl.ds(pl.multiple_of(g * G * DH, G * DH), G * DH), :]
            wo[pl.ds(pl.multiple_of(g * G * 64, G * 64), G * 64), :] = pltpu.bitcast(blk, u32)
            for j in range(VG):
                wof[g * VG + j] = blk[j * DH:(j + 1) * DH].astype(f32)

        def prep_mlp(i):
            n = FP // 2
            r = pl.ds(pl.multiple_of(i * n, 128), n)
            blk = w1t_raw[r, :].T
            w1[:, r] = pltpu.bitcast(blk, u32)
            cs1[:, r] = jnp.dot(jnp.ones((16, D), bf16), blk, preferred_element_type=f32)[0:8]
            w2[pl.ds(pl.multiple_of(i * (n // 2), 64), n // 2), :] = pltpu.bitcast(w2_raw[r, :], u32)

        def prep_rest():
            b1v = jnp.concatenate([b1_raw[...].astype(f32)[None, :], jnp.zeros((1, FP - F), f32)], axis=1)
            b1[...] = jnp.broadcast_to(b1v, (8, FP))
            b2[...] = jnp.broadcast_to(b2_raw[...].astype(f32)[None, :], (8, D))

            def rows(i):
                r = pl.multiple_of(i * 64, 64)
                w1tf[pl.ds(r, 64), :] = w1t_raw[pl.ds(fm * 128 + r, 64), :].astype(f32)
                w2f[pl.ds(r, 64), :] = w2_raw[pl.ds(fm * 128 + r, 64), :].astype(f32)
            loop(FV // 64, rows)
            for c in range(fm, FP // 128):
                n = min(128, F - c * 128)
                t = jnp.broadcast_to(b1v[:, c * 128:(c + 1) * 128], (128, 128)).T
                b1col[(c - fm) * 128:(c - fm) * 128 + n, :] = t[0:n]

        def prep_late(t):
            @pl.when(t == 0)
            def _():
                wait(w1t_raw.at[pl.ds(0, F), :], wsem.at[2])
                wait(w2_raw.at[pl.ds(0, F), :], wsem.at[3])
                w1t_raw[F:FP, :] = jnp.zeros((FP - F, D), bf16)
                w2_raw[F:FP, :] = jnp.zeros((FP - F, D), bf16)
            pl.when(t < 2)(lambda: prep_mlp(t))
            pl.when(t == 2)(prep_rest)

        loop(10, fetch_wq)
        small = [pltpu.make_async_copy(x_hbm, x_raw, wsem.at[4]),
                 pltpu.make_async_copy(b1_hbm, b1_raw, wsem.at[5]),
                 pltpu.make_async_copy(b2_hbm, b2_raw, wsem.at[6])]
        for cp in small:
            cp.start()
        loop(16, fetch_wo)
        loop(F // 64, lambda i: fetch_rows(w1t_hbm, w1t_raw, wsem.at[2], i))
        wait(wq_raw, wsem.at[0])

        def first_part(g):
            prep_wq(g)
            lax.fori_loop(7 * g, jnp.minimum(7 * g + 7, F // 64),
                          lambda i, c: (fetch_rows(w2_hbm, w2_raw, wsem.at[3], i), c)[1], 0)
        loop(NG, first_part)
        wait(wo_raw, wsem.at[1])

        def second_part(g):
            for i in range(2 * NS - behind):
                pl.when(g == i * NG // (2 * NS - behind))(lambda: stripe(i // NS, 0, i % NS))
            prep_wo(g)
        loop(NG, second_part)
        for cp in small:
            cp.wait()

        row = lax.broadcasted_iota(jnp.int32, (8, DH), 0)
        rowd = lax.broadcasted_iota(jnp.int32, (8, D), 0)
        xin[...] = x_raw[...].astype(f32)
        res[...] = jnp.zeros((8, D), f32)
        zero[...] = jnp.zeros((8, 128), jnp.int32)

        def start_layer(layer, x):
            xs[layer] = x
            accs[layer] = jnp.zeros((8, D), f32)

        def x_row(b):
            return jnp.broadcast_to(jnp.sum(jnp.where(rowd == b, xin[...], 0.0), axis=0, keepdims=True), (8, D))

        start_layer(0, x_row(0))

        def only_row(v, j):
            return unpack(pack(jnp.where(row == j, v, 0.0)))

        def queries(layer, g):
            c = pl.ds(pl.multiple_of(g * G * DH, G * DH), G * DH)
            x = xs[layer]
            m, var = moments(tiles(x))
            q = jnp.dot(jnp.concatenate([x, x], axis=0).astype(bf16), unpack(wq[:, c]),
                        preferred_element_type=f32)[0:8]
            return [t - m * cs for t, cs in zip(tiles(q), tiles(csq[:, c]))], lax.rsqrt(var + EPS) * SCALE

        def softmax(q, c, t, feed):
            s = None
            for j in range(G):
                feed()
                u = jnp.dot(only_row(q[j], j), unpack(kt[t % NV, j]), preferred_element_type=f32)[0:8]
                s = u if s is None else s + u
            s = tiles(s)
            mx = lane_max(tree(jnp.maximum, s))
            e = [jnp.exp2((u - mx) * c) for u in s]
            p = jnp.concatenate(e, axis=1)
            return jnp.concatenate([p, p], axis=0).astype(bf16), 1.0 / lane_sum(tree(jnp.add, e))

        def context(p, rl, t, js, feed=None):
            o = []
            for j in js:
                if feed:
                    feed()
                u = jnp.dot(p, unpack(v32[t % NV, j]), preferred_element_type=f32)[0:8]
                o.append(only_row(u * rl, j))
            r = ((t % NG) * G + js[0]) * 64
            r = r if isinstance(t, int) else pl.multiple_of(r, 64)
            return jnp.dot(jnp.concatenate(o, axis=1), unpack(wo[pl.ds(r, len(js) * 64), :]),
                           preferred_element_type=f32)[0:8]

        def transpose_v(t, js):
            for j in js:
                vtf[(t % NG) * VG + j] = unpack(v32[t % NV, j]).T.astype(f32)

        def after_attention(layer):
            return jnp.concatenate([a + row_sum(c) for a, c in zip(tiles(xs[layer]), tiles(accs[layer]))], axis=1)

        mlp_refs = (w1, w2, cs1, b1, b2, w1tf, w2f, b1col)

        def step(t):
            g = t % NG

            lo = jnp.where(t > LAST - 2, t + 1, t)
            hi = jnp.where(t < NG, t, jnp.minimum(jnp.where(t >= LAST - 2, t + 2, t + 1), NPAGE))

            def second_layer(u, carry):
                feed = Feed(jnp.where(u == lo, t, NPAGE), 0, 2 * G + 1)
                feed()
                p, rl = softmax(*queries(1, u % NG), u - NG, feed)
                accs[1] += context(p, rl, u - NG, range(G), feed)
                return carry
            lax.fori_loop(lo, hi, second_layer, 0)

            @pl.when(t < NG)
            def _():
                Feed(t, 0, 1)()
                prep_late(t)

            feed = Feed(t, 1, 2 * G + 1)
            wait(kbuf.at[t % NK], ksem.at[t % NK])
            feed()
            q, c = queries(0, g)
            for j in range(G):
                feed()
                kj = unpack(k32[t % NK, j]).T
                kt[t % NV, j] = pltpu.bitcast(kj, u32)
                if j < VG:
                    ktf[g * VG + j] = kj.astype(f32)
            ps[t % 2], rls[t % 2] = softmax(q, c, t, feed)

            tc = jnp.minimum(t, LAST - 1)

            @pl.when(t != LAST - 1)
            def _():
                wait(vbuf.at[tc % NV], vsem.at[tc % NV])
                transpose_v(tc, range(VG))
                accs[0] += context(ps[tc % 2], rls[tc % 2], tc, range(G), Feed(t, 2, G))

            first = (g == NG - 1) & (t < LAST)
            second = ((g == 0) & (t >= 2 * NG)) | (t == LAST - 1)

            @pl.when((first & (t >= NG)) | (t == LAST - 1))
            def _():
                xs[2] = after_attention(1)

            @pl.when(first)
            def _():
                xs[0] = after_attention(0)

            @pl.when(first | second)
            def _():
                x = mlp(tiles(xs[jnp.where(first, 0, 2)]), mlp_refs, FP // 128, Weave(None, FP, FP), 1,
                        Feed(t, 3, 4))
                x = jnp.concatenate(x, axis=1)

                @pl.when(first)
                def _():
                    start_layer(1, x)
                    start_layer(0, x_row(t // NG + 1))

                @pl.when(second)
                def _():
                    res[...] = jnp.where(rowd == (t + 2) // NG - 2, x, res[...])

            @pl.when(jnp.logical_not(first | second) & (t < LAST))
            def _():
                Feed(t, 3, 1)()

        loop(NPAGE, step)

        p, rl = ps[LAST % 2], rls[LAST % 2]
        acc = accs[0]
        for i, (lo, hi) in enumerate(zip(cuts[:-1], cuts[1:])):
            wait(vbuf.at[LAST % NV, pl.ds(lo, hi - lo)], lsem.at[i])
            transpose_v(LAST, range(lo, min(hi, vpu_heads[-1])))
            acc = acc + context(p, rl, LAST, range(lo, hi))
        xt = [a + row_sum(c) for a, c in zip(tiles(xs[0]), tiles(acc))]
        always = zero[...] == 0

        def k_half(h, hf):
            return kt[(NPAGE - NG + h // G) % NV, h % G, :, hf * 512:(hf + 1) * 512]

        def v_half(h, hf):
            return v32[(NPAGE - NG + h // G) % NV, h % G, hf * 256:(hf + 1) * 256, :]

        xt = mlp(xt, mlp_refs, fm, Weave(always, *m1[:3]), m1[3], delay=m1[4])
        xt = attention(xt, (k_half, v_half, wq, wo, csq, ktf, vtf, wqtf, wof), vheads, groups, Weave(always, *lag),
                       delays, vorder, back)
        xt = mlp(xt, mlp_refs, fm, Weave(always, *m2[:3]), m2[3], delay=m2[4])
        o_ref[...] = jnp.where(rowd == B - 1, jnp.concatenate(xt, axis=1), res[...]).astype(o_ref.dtype)

    V = pltpu.VMEM
    scratch = [
        V((NK, G, W, DH), bf16), V((NV, G, W, DH), bf16), V((NV, G, DH // 2, W), u32),
        V((NG * VG, DH, W), f32), V((NG * VG, DH, W), f32),
        V((D, H * DH), bf16), V((H * DH, D), bf16), V((FP, D), bf16), V((FP, D), bf16),
        V((B, D), bf16), V((F,), bf16), V((D,), bf16),
        V((D // 2, H * DH), u32), V((H * DH // 2, D), u32), V((D // 2, FP), u32), V((FP // 2, D), u32),
        V((NG * VG, DH, D), f32), V((NG * VG, DH, D), f32), V((FV, D), f32), V((FV, D), f32),
        V((8, H * DH), f32), V((8, FP), f32), V((8, FP), f32), V((8, D), f32), V((FV, 128), f32),
        V((8, D), f32), V((3, 8, D), f32), V((2, 8, D), f32), V((2, 16, W), bf16), V((2, 8, DH), f32),
        V((8, D), f32), V((8, 128), jnp.int32),
        pltpu.SemaphoreType.DMA((NK,)), pltpu.SemaphoreType.DMA((NV,)),
        pltpu.SemaphoreType.DMA((7,)), pltpu.SemaphoreType.DMA((len(cuts) - 1,)),
    ]

    return kernel, scratch


@jax.jit
def pallas_interleave_layers__sliding_block_cached__mixer_channel_mlp__decode_kernel(
    A_x: jax.Array,
    A_k_cache: jax.Array,
    A_v_cache: jax.Array,
    A_wq: jax.Array,
    A_wo: jax.Array,
    B_x: jax.Array,
    B_w1: jax.Array,
    B_b1: jax.Array,
    B_w2: jax.Array,
    B_b2: jax.Array,
):
    del B_x
    kernel, scratch = build_kernel()
    out = pl.pallas_call(
        kernel,
        in_specs=[pl.BlockSpec(memory_space=pltpu.HBM)] * 9,
        out_specs=pl.BlockSpec(memory_space=pltpu.VMEM),
        out_shape=jax.ShapeDtypeStruct((B, D), A_x.dtype),
        scratch_shapes=scratch,
        compiler_params=pltpu.CompilerParams(vmem_limit_bytes=124 * 1024 * 1024, disable_bounds_checks=True),
    )(A_x.reshape(B, D), A_k_cache, A_v_cache, A_wq, A_wo, B_w1.T, B_b1, B_w2, B_b2)
    return out.reshape(B, 1, D)
```

```python
import jax
import jax.numpy as jnp
from jax import lax
from jax.experimental import pallas as pl
from jax.experimental.pallas import tpu as pltpu

B, D, H, DH, SK, F = 8, 640, 32, 128, 4096, 1728
W = min(4096, max(256, SK // 4))
FP = 1792
DT = D // 128
G = 8
NG = H // G
NPAGE = B * NG
NK, NV = 4, 8
EPS = 1e-5
SCALE = DH ** -0.5 * 1.4426950408889634

LAST = NPAGE - 1

PIECE_ROWS = (64, 96) * 6 + (64,)
NS = len(PIECE_ROWS)
HEAD_ORDER = (0, 4, 3, 7, 6, 2, 1, 5)
REGIONS = (0, 4, 1, 5, 2, 6, 3, 7)
BEHIND = 5
FEED = (0, 9, 19, 21, 2 * NS)
LAST_SLOTS = [(LAST - 1, i) for i in range(23, 26)] + [(LAST, i) for i in range(9, 19)]
LAST_CUTS = (0, 6, 8)

VPU_HEADS = (4, 3, 3, 3)
MXU_GROUPS = (4, 8, 7)
VG = max(VPU_HEADS)
FM = 10
FV = F - FM * 128
JB = 4

f32, bf16, u32 = jnp.float32, jnp.bfloat16, jnp.uint32


def tiles(v):
    return [v[:, i * 128:(i + 1) * 128] for i in range(v.shape[1] // 128)]


def tree(op, xs):
    xs = list(xs)
    while len(xs) > 1:
        xs = [op(*xs[i:i + 2]) if i + 1 < len(xs) else xs[i] for i in range(0, len(xs), 2)]
    return xs[0]


def lane_sum(v):
    return jnp.broadcast_to(jnp.sum(v, axis=1, keepdims=True), v.shape)


def lane_max(v):
    return jnp.broadcast_to(jnp.max(v, axis=1, keepdims=True), v.shape)


def row_sum(v):
    return jnp.broadcast_to(jnp.sum(v, axis=0, keepdims=True), v.shape)


def accum(acc, i, val):
    acc[i] = val if acc[i] is None else acc[i] + val


def pack(a, b=None):
    return pltpu.bitcast(jnp.concatenate([a, a if b is None else b], axis=0).astype(bf16), u32)


def unpack(w):
    return pltpu.bitcast(w, bf16)


def mxu_dot(lhs, w, half=0):
    lhs = jnp.concatenate([unpack(t) for t in lhs], axis=1)
    return jnp.dot(lhs, unpack(w), preferred_element_type=f32)[half * 8:half * 8 + 8]


def moments(xt):
    m = lane_sum(tree(jnp.add, xt)) * (1.0 / D)
    sq = lane_sum(tree(jnp.add, [t * t for t in xt])) * (1.0 / D)
    return m, jnp.maximum(sq - m * m, 0.0)


def gelu(x):
    c = 0.7978845608028654
    hx = 0.5 * x
    return hx + hx * jnp.tanh(x * (c + (c * 0.044715) * (x * x)))


def loop(n, body):
    lax.fori_loop(0, n, lambda i, c: (body(i), c)[1], 0)


class Weave:
    def __init__(self, always=None, lag_m=3, lag_v=4):
        self.always, self.lag_m, self.lag_v = always, lag_m, lag_v
        self.vres, self.mres, self.fresh = [], [], False

    def tie_m(self, lhs):
        k = len(self.mres) - self.lag_m
        if k < 0 or self.vres[k] is None:
            return lhs
        return jnp.where(self.always, lhs, pltpu.bitcast(self.vres[k], u32))

    def tie_v(self, val):
        k = len(self.mres) - self.lag_v
        if k < 0 or not self.fresh:
            return val
        self.fresh = False
        return jnp.where(self.always, val, self.mres[k])

    def run(self, mxu, mxu_work, vpu, vpu_work):
        md = vd = 0
        last = None
        mxu_live, vpu_live = True, vpu_work > 0
        while mxu_live or vpu_live:
            if mxu_live and (not vpu_live or md * vpu_work <= vd * mxu_work):
                item = next(mxu, None)
                mxu_live = item is not None
                if mxu_live:
                    md += item[0]
                    self.vres.append(last)
                    self.mres.append(item[1])
                    self.fresh = True
            else:
                item = next(vpu, None)
                vpu_live = item is not None
                if vpu_live:
                    vd += item[0]
                    last = item[1]


def mlp(xt, refs, fm, feed=None):
    w1, w2, cs1, b1, b2, w1tf, w2f, b1col = refs
    m1 = lane_sum(tree(jnp.add, xt)) * (1.0 / D)
    mc, vc = moments([t - m1 for t in xt])
    r1 = lax.rsqrt(vc + mc * mc + EPS)
    r2 = lax.rsqrt(vc * r1 * r1 + EPS)
    m, r = m1 + mc, r1 * r2
    xp = [pack(xt[i], xt[min(i + 1, DT - 1)]) for i in range(0, DT, 2)]
    xc = [t - m for t in xt]
    macc, vacc = [None] * DT, [None] * DT
    chunks = [(c, min(4, fm - c)) for c in range(0, fm, 4)]
    nj = max(F - fm * 128, 0) // 8

    def mxu():
        hs = {}

        def up(i):
            c0, n = chunks[i]
            a = None
            for kb in range(DT):
                u = mxu_dot([xp[kb // 2]], w1[kb * 64:(kb + 1) * 64, c0 * 128:(c0 + n) * 128], kb % 2)
                a = u if a is None else a + u
                yield 8 * n, None
            hs[i] = []
            for j, t in enumerate(tiles(a)):
                sl = slice((c0 + j) * 128, (c0 + j + 1) * 128)
                hs[i].append(pack(gelu((t - m * cs1[:, sl]) * r + b1[:, sl])))

        def down(i):
            c0, n = chunks[i]
            for nt in range(DT):
                accum(macc, nt, mxu_dot(hs[i], w2[c0 * 64:(c0 + n) * 64, nt * 128:(nt + 1) * 128]))
                yield 8 * n, None

        for t in range(len(chunks) + 1):
            if t < len(chunks):
                if feed:
                    feed()
                yield from up(t)
            if t >= 1:
                yield from down(t - 1)

    def vpu():
        delay = 48
        col, part = {}, {}
        for step in range(nj + delay):
            if step < nj:
                blk, sub = divmod(step, JB)
                js = range(blk * JB, (blk + 1) * JB)
                for kb in range(DT):
                    if kb * JB // DT == sub:
                        for j in js:
                            t = w1tf[j * 8:(j + 1) * 8, kb * 128:(kb + 1) * 128] * xc[kb]
                            part[j] = t if kb == 0 else part[j] + t
                        yield JB, None
                if sub == JB - 1:
                    for j in js:
                        col[j] = lane_sum(part.pop(j))
            j = step - delay
            if j >= 0:
                h = gelu(col.pop(j) * r + b1col[j * 8:(j + 1) * 8, :])
                for nt in range(DT):
                    accum(vacc, nt, w2f[j * 8:(j + 1) * 8, nt * 128:(nt + 1) * 128] * h)
                yield 5, None

    Weave().run(mxu(), fm * 80, vpu(), nj * 10)
    out = []
    for nt in range(DT):
        a = xt[nt] + b2[:, nt * 128:(nt + 1) * 128] + macc[nt]
        out.append(a if vacc[nt] is None else a + row_sum(vacc[nt]))
    return out


def attention(xt, refs, vheads, groups, always):
    k_half, v_half, wq, wo, csq, ktf, vtf, wqtf, wof = refs
    weave = Weave(always)
    row = lax.broadcasted_iota(jnp.int32, (8, DH), 0)
    m, var = moments(xt)
    c = lax.rsqrt(var + EPS) * SCALE
    xc = [t - m for t in xt]
    xp = [pack(xt[i], xt[min(i + 1, DT - 1)]) for i in range(0, DT, 2)]
    macc, vacc = [None] * DT, [None] * DT

    def mxu():
        q, p, o = {}, {}, {}

        def project(g):
            for c0 in range(0, len(groups[g]), 4):
                hs = groups[g][c0:c0 + 4]
                a = None
                for kb in range(DT):
                    w = jnp.concatenate([wq[kb * 64:(kb + 1) * 64, h * 128:(h + 1) * 128] for h in hs], axis=1)
                    u = mxu_dot([weave.tie_m(xp[kb // 2])], w, kb % 2)
                    a = u if a is None else a + u
                    yield 8 * len(hs), u[:, 0:128]
                for i, t in enumerate(tiles(a)):
                    t = t - m * csq[:, hs[i] * 128:(hs[i] + 1) * 128]
                    q[g] = jnp.where(row == c0 + i, t, q[g]) if g in q else t

        def scores(g):
            s = [None] * 8
            for hf in range(2):
                for j, h in enumerate(groups[g]):
                    u = mxu_dot([weave.tie_m(pack(jnp.where(row == j, q[g], 0.0)))], k_half(h, hf))
                    for i, t in enumerate(tiles(u)):
                        accum(s, hf * 4 + i, t)
                    yield 32, u[:, 0:128]
            mx = lane_max(tree(jnp.maximum, s))
            e = [jnp.exp2((t - mx) * c) for t in s]
            p[g] = ([pack(e[i], e[i + 4]) for i in range(4)], 1.0 / lane_sum(tree(jnp.add, e)))

        def context(g):
            pk, rl = p[g]
            out = None
            for j, h in enumerate(groups[g]):
                a = None
                for hf in range(2):
                    u = mxu_dot([weave.tie_m(pk[0])] + pk[1:], v_half(h, hf), hf)
                    a = u if a is None else a + u
                    yield 32, u
                out = a if out is None else jnp.where(row == j, a, out)
            o[g] = out * rl

        def output(g):
            for c0 in range(0, len(groups[g]), 4):
                hs = groups[g][c0:c0 + 4]
                lhs = [pack(jnp.where(row == c0 + i, o[g], 0.0)) for i in range(len(hs))]
                for nt in range(DT):
                    w = jnp.concatenate([wo[h * 64:(h + 1) * 64, nt * 128:(nt + 1) * 128] for h in hs], axis=0)
                    u = mxu_dot([weave.tie_m(lhs[0])] + lhs[1:], w)
                    accum(macc, nt, u)
                    yield 8 * len(hs), u

        for t in range(len(groups) + 3):
            for d, stage in enumerate((project, scores, context, output)):
                if 0 <= t - d < len(groups):
                    yield from stage(t - d)

    def vpu():
        qcol, ocol, s, e, rl, qa, oa, seen = {}, {}, {}, {}, {}, {}, {}, {}

        def fold_rows(vals):
            low = (row & 4) == 0
            vals = [jnp.where(low, vals[k], vals[k + 4]) + pltpu.roll(jnp.where(low, vals[k + 4], vals[k]), 4, 0)
                    for k in range(4)]
            for sh in (2, 1):
                low = (row & sh) == 0
                vals = [jnp.where(low, vals[k] + pltpu.roll(vals[k], 8 - sh, 0),
                                  vals[k + sh] + pltpu.roll(vals[k + sh], sh, 0)) for k in range(sh)]
            return vals[0]

        def project(i):
            h, blk, sub = vheads[i // 16], (i % 16) // JB, i % JB
            js = range(blk * JB, (blk + 1) * JB)
            for kb in range(DT):
                if kb * JB // DT == sub:
                    x0 = weave.tie_v(xc[kb])
                    for j in js:
                        t = wqtf[h, j * 8:(j + 1) * 8, kb * 128:(kb + 1) * 128] * x0
                        qa[j] = t if kb == 0 else qa[j] + t
                    yield JB, qa[j]
            if sub == JB - 1:
                for j in js:
                    qcol[i // 16 * 16 + j] = lane_sum(qa[j])

        def scores(i):
            h, j = vheads[i // 16], i % 16
            sa = s.setdefault(h, [None] * 8)
            qc = weave.tie_v(qcol.pop(i))
            if i - 2 in seen:
                qc = jnp.where(always, qc, seen.pop(i - 2))
            for t in range(8):
                accum(sa, t, ktf[h, j * 8:(j + 1) * 8, t * 128:(t + 1) * 128] * qc)
            seen[i] = sa[0]
            if j == 15:
                sc = fold_rows(s.pop(h))
                mx = lane_max(jnp.broadcast_to(jnp.max(sc, axis=0, keepdims=True), sc.shape))
                e[h] = jnp.exp2((sc - mx) * c)
                rl[h] = 1.0 / lane_sum(row_sum(e[h]))
            yield 8, sa[7]

        def context(i):
            h, blk, sub = vheads[i // 16], (i % 16) // JB, i % JB
            js = range(blk * JB, (blk + 1) * JB)
            for t in range(8):
                if t * JB // 8 == sub:
                    e0 = weave.tie_v(jnp.broadcast_to(e[h][t:t + 1, :], (8, DH)))
                    for j in js:
                        u = vtf[h, j * 8:(j + 1) * 8, t * 128:(t + 1) * 128] * e0
                        oa[j] = u if t == 0 else oa[j] + u
                    yield JB, oa[j]
            if sub == JB - 1:
                for j in js:
                    ocol[i // 16 * 16 + j] = lane_sum(oa[j]) * rl[h]

        def output(i):
            h, j = vheads[i // 16], i % 16
            oc = weave.tie_v(ocol.pop(i))
            for nt in range(DT):
                accum(vacc, nt, wof[h, j * 8:(j + 1) * 8, nt * 128:(nt + 1) * 128] * oc)
            yield 5, vacc[DT - 1]

        n = len(vheads) * 16
        stages = ((project, 0), (scores, 10), (context, 36), (output, 48))
        for step in range(n + stages[-1][1]):
            for stage, delay in stages:
                if 0 <= step - delay < n:
                    yield from stage(step - delay)

    weave.run(mxu(), sum(len(g) for g in groups) * 208, vpu(), len(vheads) * 416)
    return [xt[nt] + row_sum(macc[nt] + vacc[nt]) for nt in range(DT)]


def build_kernel():
    vheads = [g * VG + j for g in range(NG) for j in range(VPU_HEADS[g])]
    mheads = [g * G + j for g in range(NG) for j in range(VPU_HEADS[g], G)]
    groups = [mheads[sum(MXU_GROUPS[:i]):sum(MXU_GROUPS[:i + 1])] for i in range(len(MXU_GROUPS))]

    def kernel(x_hbm, k_hbm, v_hbm, wq_hbm, wo_hbm, w1t_hbm, b1_hbm, w2_hbm, b2_hbm, o_ref,
               kbuf, vbuf, kt, ktf, vtf,
               wq_raw, wo_raw, w1t_raw, w2_raw, x_raw, b1_raw, b2_raw,
               wq, wo, w1, w2, wqtf, wof, w1tf, w2f, csq, cs1, b1, b2, b1col,
               xin, xs, accs, ps, rls, res, zero, ksem, vsem, wsem, lsem):
        k32, v32 = kbuf.bitcast(u32), vbuf.bitcast(u32)

        def piece(src, buf, sem, t, hh, n, queue):
            r, size = sum(PIECE_ROWS[:n]), PIECE_ROWS[n]
            pltpu.make_async_copy(
                src.at[t // NG, (t % NG) * G + hh, pl.ds(SK - W + r, size), :],
                buf.at[t % buf.shape[0], hh, pl.ds(r, size), :], sem).start(priority=queue)

        def stripe(is_v, t, n):
            src, buf, sem = ((k_hbm, kbuf, ksem), (v_hbm, vbuf, vsem))[is_v]
            for i, hh in enumerate(HEAD_ORDER):
                piece(src, buf, sem.at[t % buf.shape[0]], t, hh, n, i % 2)

        def last_stripe(i):
            order = [(h + k * (G // 2), n) for h in range(G // 2) for n in range(NS) for k in range(2)]
            for hh, n in order[i * G:(i + 1) * G]:
                part = sum(hh >= c for c in LAST_CUTS[1:-1])
                piece(v_hbm, vbuf, lsem.at[part], LAST, hh, n, hh // (G // 2))

        def slot(t, i):
            for n, (tt, ii) in enumerate(LAST_SLOTS):
                if ii == i:
                    pl.when(t == tt)(lambda: last_stripe(n))
            wrap, i = divmod(i - BEHIND, 2 * NS)
            is_v, n = divmod(i, NS)
            page = t + 1 + wrap
            swapped = LAST - is_v
            pl.when(page < swapped)(lambda: stripe(is_v, page, n))
            pl.when(page == swapped)(lambda: stripe(1 - is_v, LAST - 1 + is_v, n))

        class Feed:
            def __init__(self, t, part, calls):
                self.t, self.lo, self.n, self.calls, self.k = t, FEED[part], FEED[part + 1] - FEED[part], calls, 0

            def __call__(self):
                a, e = (self.lo - (-self.n * k // self.calls) for k in (self.k, self.k + 1))
                self.k += 1
                for i in range(a, e):
                    slot(self.t, i)

        def wait(ref, sem):
            pltpu.make_async_copy(ref, ref, sem).wait()

        def fetch_wq(i):
            c = 0
            for n in (8 * 128, 12 * 128, 12 * 128):
                for k, h in enumerate(REGIONS):
                    at = (pl.ds(pl.multiple_of((h * 10 + i) * 8, 8), 8), pl.ds(c, n))
                    pltpu.make_async_copy(wq_hbm.at[at], wq_raw.at[at], wsem.at[0]).start(priority=k % 2)
                c += n

        def fetch_wo(i):
            for r, n in ((0, 8), (8, 24)):
                for k, h in enumerate(REGIONS):
                    at = pl.ds(pl.multiple_of(h * 512 + i * 32 + r, 8), n)
                    pltpu.make_async_copy(wo_hbm.at[at, :], wo_raw.at[at, :], wsem.at[1]).start(priority=k % 2)

        def fetch_rows(src, dst, sem, i):
            for r in (0, 16):
                for q in range(2):
                    at = pl.ds(pl.multiple_of(i * 32 + r + q * (F // 2), 16), 16)
                    pltpu.make_async_copy(src.at[at, :], dst.at[at, :], sem).start(priority=q)

        def prep_wq(g):
            c = pl.ds(pl.multiple_of(g * G * DH, G * DH), G * DH)
            blk = wq_raw[:, c]
            wq[:, c] = pltpu.bitcast(blk, u32)
            csq[:, c] = jnp.dot(jnp.ones((16, D), bf16), blk, preferred_element_type=f32)[0:8]
            for j in range(VG):
                wqtf[g * VG + j] = blk[:, j * DH:(j + 1) * DH].T.astype(f32)

        def prep_wo(g):
            blk = wo_raw[pl.ds(pl.multiple_of(g * G * DH, G * DH), G * DH), :]
            wo[pl.ds(pl.multiple_of(g * G * 64, G * 64), G * 64), :] = pltpu.bitcast(blk, u32)
            for j in range(VG):
                wof[g * VG + j] = blk[j * DH:(j + 1) * DH].astype(f32)

        def prep_mlp(i):
            n = FP // 2
            r = pl.ds(pl.multiple_of(i * n, 128), n)
            blk = w1t_raw[r, :].T
            w1[:, r] = pltpu.bitcast(blk, u32)
            cs1[:, r] = jnp.dot(jnp.ones((16, D), bf16), blk, preferred_element_type=f32)[0:8]
            w2[pl.ds(pl.multiple_of(i * (n // 2), 64), n // 2), :] = pltpu.bitcast(w2_raw[r, :], u32)

        def prep_rest():
            b1v = jnp.concatenate([b1_raw[...].astype(f32)[None, :], jnp.zeros((1, FP - F), f32)], axis=1)
            b1[...] = jnp.broadcast_to(b1v, (8, FP))
            b2[...] = jnp.broadcast_to(b2_raw[...].astype(f32)[None, :], (8, D))

            def rows(i):
                r = pl.multiple_of(i * 64, 64)
                w1tf[pl.ds(r, 64), :] = w1t_raw[pl.ds(FM * 128 + r, 64), :].astype(f32)
                w2f[pl.ds(r, 64), :] = w2_raw[pl.ds(FM * 128 + r, 64), :].astype(f32)
            loop(FV // 64, rows)
            for c in range(FM, FP // 128):
                n = min(128, F - c * 128)
                t = jnp.broadcast_to(b1v[:, c * 128:(c + 1) * 128], (128, 128)).T
                b1col[(c - FM) * 128:(c - FM) * 128 + n, :] = t[0:n]

        def prep_late(t):
            @pl.when(t == 0)
            def _():
                wait(w1t_raw.at[pl.ds(0, F), :], wsem.at[2])
                wait(w2_raw.at[pl.ds(0, F), :], wsem.at[3])
                w1t_raw[F:FP, :] = jnp.zeros((FP - F, D), bf16)
                w2_raw[F:FP, :] = jnp.zeros((FP - F, D), bf16)
            pl.when(t < 2)(lambda: prep_mlp(t))
            pl.when(t == 2)(prep_rest)

        loop(10, fetch_wq)
        small = [pltpu.make_async_copy(x_hbm, x_raw, wsem.at[4]),
                 pltpu.make_async_copy(b1_hbm, b1_raw, wsem.at[5]),
                 pltpu.make_async_copy(b2_hbm, b2_raw, wsem.at[6])]
        for cp in small:
            cp.start()
        loop(16, fetch_wo)
        loop(F // 64, lambda i: fetch_rows(w1t_hbm, w1t_raw, wsem.at[2], i))
        wait(wq_raw, wsem.at[0])

        def first_part(g):
            prep_wq(g)
            lax.fori_loop(7 * g, jnp.minimum(7 * g + 7, F // 64),
                          lambda i, c: (fetch_rows(w2_hbm, w2_raw, wsem.at[3], i), c)[1], 0)
        loop(NG, first_part)
        wait(wo_raw, wsem.at[1])

        def second_part(g):
            for i in range(2 * NS - BEHIND):
                pl.when(g == i * NG // (2 * NS - BEHIND))(lambda: stripe(i // NS, 0, i % NS))
            prep_wo(g)
        loop(NG, second_part)
        for cp in small:
            cp.wait()

        row = lax.broadcasted_iota(jnp.int32, (8, DH), 0)
        rowd = lax.broadcasted_iota(jnp.int32, (8, D), 0)
        xin[...] = x_raw[...].astype(f32)
        res[...] = jnp.zeros((8, D), f32)
        zero[...] = jnp.zeros((8, 128), jnp.int32)

        def start_layer(layer, x):
            xs[layer] = x
            accs[layer] = jnp.zeros((8, D), f32)

        def x_row(b):
            return jnp.broadcast_to(jnp.sum(jnp.where(rowd == b, xin[...], 0.0), axis=0, keepdims=True), (8, D))

        start_layer(0, x_row(0))

        def only_row(v, j):
            return unpack(pack(jnp.where(row == j, v, 0.0)))

        def queries(layer, g):
            c = pl.ds(pl.multiple_of(g * G * DH, G * DH), G * DH)
            x = xs[layer]
            m, var = moments(tiles(x))
            q = jnp.dot(jnp.concatenate([x, x], axis=0).astype(bf16), unpack(wq[:, c]),
                        preferred_element_type=f32)[0:8]
            return [t - m * cs for t, cs in zip(tiles(q), tiles(csq[:, c]))], lax.rsqrt(var + EPS) * SCALE

        def softmax(q, c, t, feed):
            s = None
            for j in range(G):
                feed()
                u = jnp.dot(only_row(q[j], j), unpack(kt[t % NV, j]), preferred_element_type=f32)[0:8]
                s = u if s is None else s + u
            s = tiles(s)
            mx = lane_max(tree(jnp.maximum, s))
            e = [jnp.exp2((u - mx) * c) for u in s]
            p = jnp.concatenate(e, axis=1)
            return jnp.concatenate([p, p], axis=0).astype(bf16), 1.0 / lane_sum(tree(jnp.add, e))

        def context(p, rl, t, js, feed=None):
            o = []
            for j in js:
                if feed:
                    feed()
                u = jnp.dot(p, unpack(v32[t % NV, j]), preferred_element_type=f32)[0:8]
                o.append(only_row(u * rl, j))
            r = ((t % NG) * G + js[0]) * 64
            r = r if isinstance(t, int) else pl.multiple_of(r, 64)
            return jnp.dot(jnp.concatenate(o, axis=1), unpack(wo[pl.ds(r, len(js) * 64), :]),
                           preferred_element_type=f32)[0:8]

        def transpose_v(t, js):
            for j in js:
                vtf[(t % NG) * VG + j] = unpack(v32[t % NV, j]).T.astype(f32)

        def after_attention(layer):
            return jnp.concatenate([a + row_sum(c) for a, c in zip(tiles(xs[layer]), tiles(accs[layer]))], axis=1)

        mlp_refs = (w1, w2, cs1, b1, b2, w1tf, w2f, b1col)

        def step(t):
            g = t % NG

            lo = jnp.where(t > LAST - 2, t + 1, t)
            hi = jnp.where(t < NG, t, jnp.minimum(jnp.where(t >= LAST - 2, t + 2, t + 1), NPAGE))

            def second_layer(u, carry):
                feed = Feed(jnp.where(u == lo, t, NPAGE), 0, 2 * G + 1)
                feed()
                p, rl = softmax(*queries(1, u % NG), u - NG, feed)
                accs[1] += context(p, rl, u - NG, range(G), feed)
                return carry
            lax.fori_loop(lo, hi, second_layer, 0)

            @pl.when(t < NG)
            def _():
                Feed(t, 0, 1)()
                prep_late(t)

            feed = Feed(t, 1, 2 * G + 1)
            wait(kbuf.at[t % NK], ksem.at[t % NK])
            feed()
            q, c = queries(0, g)
            for j in range(G):
                feed()
                kj = unpack(k32[t % NK, j]).T
                kt[t % NV, j] = pltpu.bitcast(kj, u32)
                if j < VG:
                    ktf[g * VG + j] = kj.astype(f32)
            ps[t % 2], rls[t % 2] = softmax(q, c, t, feed)

            tc = jnp.minimum(t, LAST - 1)

            @pl.when(t != LAST - 1)
            def _():
                wait(vbuf.at[tc % NV], vsem.at[tc % NV])
                transpose_v(tc, range(VG))
                accs[0] += context(ps[tc % 2], rls[tc % 2], tc, range(G), Feed(t, 2, G))

            first = (g == NG - 1) & (t < LAST)
            second = ((g == 0) & (t >= 2 * NG)) | (t == LAST - 1)

            @pl.when((first & (t >= NG)) | (t == LAST - 1))
            def _():
                xs[2] = after_attention(1)

            @pl.when(first)
            def _():
                xs[0] = after_attention(0)

            @pl.when(first | second)
            def _():
                x = mlp(tiles(xs[jnp.where(first, 0, 2)]), mlp_refs, FP // 128, Feed(t, 3, 4))
                x = jnp.concatenate(x, axis=1)

                @pl.when(first)
                def _():
                    start_layer(1, x)
                    start_layer(0, x_row(t // NG + 1))

                @pl.when(second)
                def _():
                    res[...] = jnp.where(rowd == (t + 2) // NG - 2, x, res[...])

            @pl.when(jnp.logical_not(first | second) & (t < LAST))
            def _():
                Feed(t, 3, 1)()

        loop(NPAGE, step)

        p, rl = ps[LAST % 2], rls[LAST % 2]
        acc = accs[0]
        for i, (lo, hi) in enumerate(zip(LAST_CUTS[:-1], LAST_CUTS[1:])):
            wait(vbuf.at[LAST % NV, pl.ds(lo, hi - lo)], lsem.at[i])
            transpose_v(LAST, range(lo, min(hi, VPU_HEADS[-1])))
            acc = acc + context(p, rl, LAST, range(lo, hi))
        xt = [a + row_sum(c) for a, c in zip(tiles(xs[0]), tiles(acc))]
        always = zero[...] == 0

        def k_half(h, hf):
            return kt[(NPAGE - NG + h // G) % NV, h % G, :, hf * 512:(hf + 1) * 512]

        def v_half(h, hf):
            return v32[(NPAGE - NG + h // G) % NV, h % G, hf * 256:(hf + 1) * 256, :]

        xt = mlp(xt, mlp_refs, FM)
        xt = attention(xt, (k_half, v_half, wq, wo, csq, ktf, vtf, wqtf, wof), vheads, groups, always)
        xt = mlp(xt, mlp_refs, FM)
        o_ref[...] = jnp.where(rowd == B - 1, jnp.concatenate(xt, axis=1), res[...]).astype(o_ref.dtype)

    V = pltpu.VMEM
    scratch = [
        V((NK, G, W, DH), bf16), V((NV, G, W, DH), bf16), V((NV, G, DH // 2, W), u32),
        V((NG * VG, DH, W), f32), V((NG * VG, DH, W), f32),
        V((D, H * DH), bf16), V((H * DH, D), bf16), V((FP, D), bf16), V((FP, D), bf16),
        V((B, D), bf16), V((F,), bf16), V((D,), bf16),
        V((D // 2, H * DH), u32), V((H * DH // 2, D), u32), V((D // 2, FP), u32), V((FP // 2, D), u32),
        V((NG * VG, DH, D), f32), V((NG * VG, DH, D), f32), V((FV, D), f32), V((FV, D), f32),
        V((8, H * DH), f32), V((8, FP), f32), V((8, FP), f32), V((8, D), f32), V((FV, 128), f32),
        V((8, D), f32), V((3, 8, D), f32), V((2, 8, D), f32), V((2, 16, W), bf16), V((2, 8, DH), f32),
        V((8, D), f32), V((8, 128), jnp.int32),
        pltpu.SemaphoreType.DMA((NK,)), pltpu.SemaphoreType.DMA((NV,)),
        pltpu.SemaphoreType.DMA((7,)), pltpu.SemaphoreType.DMA((len(LAST_CUTS) - 1,)),
    ]

    return kernel, scratch


@jax.jit
def pallas_interleave_layers__sliding_block_cached__mixer_channel_mlp__decode_kernel(
    A_x: jax.Array,
    A_k_cache: jax.Array,
    A_v_cache: jax.Array,
    A_wq: jax.Array,
    A_wo: jax.Array,
    B_x: jax.Array,
    B_w1: jax.Array,
    B_b1: jax.Array,
    B_w2: jax.Array,
    B_b2: jax.Array,
):
    del B_x
    kernel, scratch = build_kernel()
    out = pl.pallas_call(
        kernel,
        in_specs=[pl.BlockSpec(memory_space=pltpu.HBM)] * 9,
        out_specs=pl.BlockSpec(memory_space=pltpu.VMEM),
        out_shape=jax.ShapeDtypeStruct((B, D), A_x.dtype),
        scratch_shapes=scratch,
        compiler_params=pltpu.CompilerParams(vmem_limit_bytes=124 * 1024 * 1024, disable_bounds_checks=True),
    )(A_x.reshape(B, D), A_k_cache, A_v_cache, A_wq, A_wo, B_w1.T, B_b1, B_w2, B_b2)
    return out.reshape(B, 1, D)
```

```python
import jax
import jax.numpy as jnp
from jax import lax
from jax.experimental import pallas as pl
from jax.experimental.pallas import tpu as pltpu

B, D, H, DH, SK, F = 8, 640, 32, 128, 4096, 1728
W = min(4096, max(256, SK // 4))
FP = 1792
DT = D // 128
G = 8
NG = H // G
NPAGE = B * NG
NK, NV = 4, 8
EPS = 1e-5
SCALE = DH ** -0.5 * 1.4426950408889634

LAST = NPAGE - 1

PIECE_ROWS = (64, 96) * 6 + (64,)
NS = len(PIECE_ROWS)
HEAD_ORDER = (0, 4, 3, 7, 6, 2, 1, 5)
REGIONS = (0, 4, 1, 5, 2, 6, 3, 7)
BEHIND = 5
FEED = (0, 9, 19, 21, 2 * NS)
LAST_SLOTS = [(LAST - 1, i) for i in range(23, 26)] + [(LAST, i) for i in range(9, 19)]
LAST_CUTS = (0, 6, 8)

VPU_HEADS = (4, 3, 3, 3)
MXU_GROUPS = (4, 8, 7)
VG = max(VPU_HEADS)
FM = 10
FV = F - FM * 128
JB = 4

f32, bf16, u32 = jnp.float32, jnp.bfloat16, jnp.uint32


def tiles(v):
    return [v[:, i * 128:(i + 1) * 128] for i in range(v.shape[1] // 128)]


def tree(op, xs):
    xs = list(xs)
    while len(xs) > 1:
        xs = [op(*xs[i:i + 2]) if i + 1 < len(xs) else xs[i] for i in range(0, len(xs), 2)]
    return xs[0]


def lane_sum(v):
    return jnp.broadcast_to(jnp.sum(v, axis=1, keepdims=True), v.shape)


def lane_max(v):
    return jnp.broadcast_to(jnp.max(v, axis=1, keepdims=True), v.shape)


def row_sum(v):
    return jnp.broadcast_to(jnp.sum(v, axis=0, keepdims=True), v.shape)


def accum(acc, i, val):
    acc[i] = val if acc[i] is None else acc[i] + val


def pack(a, b=None):
    return pltpu.bitcast(jnp.concatenate([a, a if b is None else b], axis=0).astype(bf16), u32)


def unpack(w):
    return pltpu.bitcast(w, bf16)


def mxu_dot(lhs, w, half=0):
    lhs = jnp.concatenate([unpack(t) for t in lhs], axis=1)
    return jnp.dot(lhs, unpack(w), preferred_element_type=f32)[half * 8:half * 8 + 8]


def moments(xt):
    m = lane_sum(tree(jnp.add, xt)) * (1.0 / D)
    sq = lane_sum(tree(jnp.add, [t * t for t in xt])) * (1.0 / D)
    return m, jnp.maximum(sq - m * m, 0.0)


def gelu(x):
    c = 0.7978845608028654
    hx = 0.5 * x
    return hx + hx * jnp.tanh(x * (c + (c * 0.044715) * (x * x)))


def loop(n, body):
    lax.fori_loop(0, n, lambda i, c: (body(i), c)[1], 0)


class Weave:
    def __init__(self, always=None, lag_m=3, lag_v=4):
        self.always, self.lag_m, self.lag_v = always, lag_m, lag_v
        self.vres, self.mres, self.fresh = [], [], False

    def tie_m(self, lhs):
        k = len(self.mres) - self.lag_m
        if k < 0 or self.vres[k] is None:
            return lhs
        return jnp.where(self.always, lhs, pltpu.bitcast(self.vres[k], u32))

    def tie_v(self, val):
        k = len(self.mres) - self.lag_v
        if k < 0 or not self.fresh:
            return val
        self.fresh = False
        return jnp.where(self.always, val, self.mres[k])

    def run(self, mxu, mxu_work, vpu, vpu_work):
        md = vd = 0
        last = None
        mxu_live, vpu_live = True, vpu_work > 0
        while mxu_live or vpu_live:
            if mxu_live and (not vpu_live or md * vpu_work <= vd * mxu_work):
                item = next(mxu, None)
                mxu_live = item is not None
                if mxu_live:
                    md += item[0]
                    self.vres.append(last)
                    self.mres.append(item[1])
                    self.fresh = True
            else:
                item = next(vpu, None)
                vpu_live = item is not None
                if vpu_live:
                    vd += item[0]
                    last = item[1]


def mlp(xt, refs, fm, feed=None):
    w1, w2, cs1, b1, b2, w1tf, w2f, b1col, cs1col = refs
    m1 = lane_sum(tree(jnp.add, xt)) * (1.0 / D)
    xc = [t - m1 for t in xt]
    mc, vc = moments(xc)
    r1 = lax.rsqrt(vc + mc * mc + EPS)
    r2 = lax.rsqrt(vc * r1 * r1 + EPS)
    m, r = m1 + mc, r1 * r2
    xp = [pack(xt[i], xt[min(i + 1, DT - 1)]) for i in range(0, DT, 2)]
    macc, vacc = [None] * DT, [None] * DT
    chunks = [(c, min(4, fm - c)) for c in range(0, fm, 4)]
    nj = max(F - fm * 128, 0) // 8

    def mxu():
        hs = {}

        def up(i):
            c0, n = chunks[i]
            a = None
            for kb in range(DT):
                u = mxu_dot([xp[kb // 2]], w1[kb * 64:(kb + 1) * 64, c0 * 128:(c0 + n) * 128], kb % 2)
                a = u if a is None else a + u
                yield 8 * n, None
            hs[i] = []
            for j, t in enumerate(tiles(a)):
                sl = slice((c0 + j) * 128, (c0 + j + 1) * 128)
                hs[i].append(pack(gelu((t - m * cs1[:, sl]) * r + b1[:, sl])))

        def down(i):
            c0, n = chunks[i]
            for nt in range(DT):
                accum(macc, nt, mxu_dot(hs[i], w2[c0 * 64:(c0 + n) * 64, nt * 128:(nt + 1) * 128]))
                yield 8 * n, None

        for t in range(len(chunks) + 1):
            if t < len(chunks):
                if feed:
                    feed()
                yield from up(t)
            if t >= 1:
                yield from down(t - 1)

    def vpu():
        delay = 48
        col, part = {}, {}
        for step in range(nj + delay):
            if step < nj:
                blk, sub = divmod(step, JB)
                js = range(blk * JB, (blk + 1) * JB)
                for kb in range(DT):
                    if kb * JB // DT == sub:
                        for j in js:
                            t = w1tf[j * 8:(j + 1) * 8, kb * 128:(kb + 1) * 128] * xc[kb]
                            part[j] = t if kb == 0 else part[j] + t
                        yield JB, None
                if sub == JB - 1:
                    for j in js:
                        col[j] = lane_sum(part.pop(j))
            j = step - delay
            if j >= 0:
                sl = slice(j * 8, (j + 1) * 8)
                h = gelu((col.pop(j) - mc * cs1col[sl, :]) * r + b1col[sl, :])
                for nt in range(DT):
                    accum(vacc, nt, w2f[j * 8:(j + 1) * 8, nt * 128:(nt + 1) * 128] * h)
                yield 5, None

    Weave().run(mxu(), fm * 80, vpu(), nj * 10)
    out = []
    for nt in range(DT):
        a = xt[nt] + b2[:, nt * 128:(nt + 1) * 128] + macc[nt]
        out.append(a if vacc[nt] is None else a + row_sum(vacc[nt]))
    return out


def attention(xt, refs, vheads, groups, always):
    k_half, v_half, wq, wo, csq, ktf, vtf, wqtf, wof = refs
    weave = Weave(always)
    row = lax.broadcasted_iota(jnp.int32, (8, DH), 0)
    m, var = moments(xt)
    c = lax.rsqrt(var + EPS) * SCALE
    xc = [t - m for t in xt]
    xp = [pack(xt[i], xt[min(i + 1, DT - 1)]) for i in range(0, DT, 2)]
    macc, vacc = [None] * DT, [None] * DT

    def mxu():
        q, p, o = {}, {}, {}

        def project(g):
            for c0 in range(0, len(groups[g]), 4):
                hs = groups[g][c0:c0 + 4]
                a = None
                for kb in range(DT):
                    w = jnp.concatenate([wq[kb * 64:(kb + 1) * 64, h * 128:(h + 1) * 128] for h in hs], axis=1)
                    u = mxu_dot([weave.tie_m(xp[kb // 2])], w, kb % 2)
                    a = u if a is None else a + u
                    yield 8 * len(hs), u[:, 0:128]
                for i, t in enumerate(tiles(a)):
                    t = t - m * csq[:, hs[i] * 128:(hs[i] + 1) * 128]
                    q[g] = jnp.where(row == c0 + i, t, q[g]) if g in q else t

        def scores(g):
            s = [None] * 8
            for hf in range(2):
                for j, h in enumerate(groups[g]):
                    u = mxu_dot([weave.tie_m(pack(jnp.where(row == j, q[g], 0.0)))], k_half(h, hf))
                    for i, t in enumerate(tiles(u)):
                        accum(s, hf * 4 + i, t)
                    yield 32, u[:, 0:128]
            mx = lane_max(tree(jnp.maximum, s))
            e = [jnp.exp2((t - mx) * c) for t in s]
            p[g] = ([pack(e[i], e[i + 4]) for i in range(4)], 1.0 / lane_sum(tree(jnp.add, e)))

        def context(g):
            pk, rl = p[g]
            out = None
            for j, h in enumerate(groups[g]):
                a = None
                for hf in range(2):
                    u = mxu_dot([weave.tie_m(pk[0])] + pk[1:], v_half(h, hf), hf)
                    a = u if a is None else a + u
                    yield 32, u
                out = a if out is None else jnp.where(row == j, a, out)
            o[g] = out * rl

        def output(g):
            for c0 in range(0, len(groups[g]), 4):
                hs = groups[g][c0:c0 + 4]
                lhs = [pack(jnp.where(row == c0 + i, o[g], 0.0)) for i in range(len(hs))]
                for nt in range(DT):
                    w = jnp.concatenate([wo[h * 64:(h + 1) * 64, nt * 128:(nt + 1) * 128] for h in hs], axis=0)
                    u = mxu_dot([weave.tie_m(lhs[0])] + lhs[1:], w)
                    accum(macc, nt, u)
                    yield 8 * len(hs), u

        for t in range(len(groups) + 3):
            for d, stage in enumerate((project, scores, context, output)):
                if 0 <= t - d < len(groups):
                    yield from stage(t - d)

    def vpu():
        qcol, ocol, s, e, rl, qa, oa, seen = {}, {}, {}, {}, {}, {}, {}, {}

        def fold_rows(vals):
            low = (row & 4) == 0
            vals = [jnp.where(low, vals[k], vals[k + 4]) + pltpu.roll(jnp.where(low, vals[k + 4], vals[k]), 4, 0)
                    for k in range(4)]
            for sh in (2, 1):
                low = (row & sh) == 0
                vals = [jnp.where(low, vals[k] + pltpu.roll(vals[k], 8 - sh, 0),
                                  vals[k + sh] + pltpu.roll(vals[k + sh], sh, 0)) for k in range(sh)]
            return vals[0]

        def project(i):
            h, blk, sub = vheads[i // 16], (i % 16) // JB, i % JB
            js = range(blk * JB, (blk + 1) * JB)
            for kb in range(DT):
                if kb * JB // DT == sub:
                    x0 = weave.tie_v(xc[kb])
                    for j in js:
                        t = wqtf[h, j * 8:(j + 1) * 8, kb * 128:(kb + 1) * 128] * x0
                        qa[j] = t if kb == 0 else qa[j] + t
                    yield JB, qa[j]
            if sub == JB - 1:
                for j in js:
                    qcol[i // 16 * 16 + j] = lane_sum(qa[j])

        def scores(i):
            h, j = vheads[i // 16], i % 16
            sa = s.setdefault(h, [None] * 8)
            qc = weave.tie_v(qcol.pop(i))
            if i - 2 in seen:
                qc = jnp.where(always, qc, seen.pop(i - 2))
            for t in range(8):
                accum(sa, t, ktf[h, j * 8:(j + 1) * 8, t * 128:(t + 1) * 128] * qc)
            seen[i] = sa[0]
            if j == 15:
                sc = fold_rows(s.pop(h))
                mx = lane_max(jnp.broadcast_to(jnp.max(sc, axis=0, keepdims=True), sc.shape))
                e[h] = jnp.exp2((sc - mx) * c)
                rl[h] = 1.0 / lane_sum(row_sum(e[h]))
            yield 8, sa[7]

        def context(i):
            h, blk, sub = vheads[i // 16], (i % 16) // JB, i % JB
            js = range(blk * JB, (blk + 1) * JB)
            for t in range(8):
                if t * JB // 8 == sub:
                    e0 = weave.tie_v(jnp.broadcast_to(e[h][t:t + 1, :], (8, DH)))
                    for j in js:
                        u = vtf[h, j * 8:(j + 1) * 8, t * 128:(t + 1) * 128] * e0
                        oa[j] = u if t == 0 else oa[j] + u
                    yield JB, oa[j]
            if sub == JB - 1:
                for j in js:
                    ocol[i // 16 * 16 + j] = lane_sum(oa[j]) * rl[h]

        def output(i):
            h, j = vheads[i // 16], i % 16
            oc = weave.tie_v(ocol.pop(i))
            for nt in range(DT):
                accum(vacc, nt, wof[h, j * 8:(j + 1) * 8, nt * 128:(nt + 1) * 128] * oc)
            yield 5, vacc[DT - 1]

        n = len(vheads) * 16
        stages = ((project, 0), (scores, 10), (context, 36), (output, 48))
        for step in range(n + stages[-1][1]):
            for stage, delay in stages:
                if 0 <= step - delay < n:
                    yield from stage(step - delay)

    weave.run(mxu(), sum(len(g) for g in groups) * 208, vpu(), len(vheads) * 416)
    return [xt[nt] + row_sum(macc[nt] + vacc[nt]) for nt in range(DT)]


def build_kernel():
    vheads = [g * VG + j for g in range(NG) for j in range(VPU_HEADS[g])]
    mheads = [g * G + j for g in range(NG) for j in range(VPU_HEADS[g], G)]
    groups = [mheads[sum(MXU_GROUPS[:i]):sum(MXU_GROUPS[:i + 1])] for i in range(len(MXU_GROUPS))]

    def kernel(x_hbm, k_hbm, v_hbm, wq_hbm, wo_hbm, w1t_hbm, b1_hbm, w2_hbm, b2_hbm, o_ref,
               kbuf, vbuf, kt, ktf, vtf,
               wq_raw, wo_raw, w1t_raw, w2_raw, x_raw, b1_raw, b2_raw,
               wq, wo, w1, w2, wqtf, wof, w1tf, w2f, csq, cs1, b1, b2, b1col, cs1col,
               xin, xs, accs, ps, rls, res, zero, ksem, vsem, wsem, lsem):
        k32, v32 = kbuf.bitcast(u32), vbuf.bitcast(u32)

        def piece(src, buf, sem, t, hh, n, queue):
            r, size = sum(PIECE_ROWS[:n]), PIECE_ROWS[n]
            pltpu.make_async_copy(
                src.at[t // NG, (t % NG) * G + hh, pl.ds(SK - W + r, size), :],
                buf.at[t % buf.shape[0], hh, pl.ds(r, size), :], sem).start(priority=queue)

        def stripe(is_v, t, n):
            src, buf, sem = ((k_hbm, kbuf, ksem), (v_hbm, vbuf, vsem))[is_v]
            for i, hh in enumerate(HEAD_ORDER):
                piece(src, buf, sem.at[t % buf.shape[0]], t, hh, n, i % 2)

        def last_stripe(i):
            order = [(h + k * (G // 2), n) for h in range(G // 2) for n in range(NS) for k in range(2)]
            for hh, n in order[i * G:(i + 1) * G]:
                part = sum(hh >= c for c in LAST_CUTS[1:-1])
                piece(v_hbm, vbuf, lsem.at[part], LAST, hh, n, hh // (G // 2))

        def slot(t, i):
            for n, (tt, ii) in enumerate(LAST_SLOTS):
                if ii == i:
                    pl.when(t == tt)(lambda: last_stripe(n))
            wrap, i = divmod(i - BEHIND, 2 * NS)
            is_v, n = divmod(i, NS)
            page = t + 1 + wrap
            swapped = LAST - is_v
            pl.when(page < swapped)(lambda: stripe(is_v, page, n))
            pl.when(page == swapped)(lambda: stripe(1 - is_v, LAST - 1 + is_v, n))

        class Feed:
            def __init__(self, t, part, calls):
                self.t, self.lo, self.n, self.calls, self.k = t, FEED[part], FEED[part + 1] - FEED[part], calls, 0

            def __call__(self):
                a, e = (self.lo - (-self.n * k // self.calls) for k in (self.k, self.k + 1))
                self.k += 1
                for i in range(a, e):
                    slot(self.t, i)

        def wait(ref, sem):
            pltpu.make_async_copy(ref, ref, sem).wait()

        def fetch_wq(i):
            c = 0
            for n in (8 * 128, 12 * 128, 12 * 128):
                for k, h in enumerate(REGIONS):
                    at = (pl.ds(pl.multiple_of((h * 10 + i) * 8, 8), 8), pl.ds(c, n))
                    pltpu.make_async_copy(wq_hbm.at[at], wq_raw.at[at], wsem.at[0]).start(priority=k % 2)
                c += n

        def fetch_wo(i):
            for r, n in ((0, 8), (8, 24)):
                for k, h in enumerate(REGIONS):
                    at = pl.ds(pl.multiple_of(h * 512 + i * 32 + r, 8), n)
                    pltpu.make_async_copy(wo_hbm.at[at, :], wo_raw.at[at, :], wsem.at[1]).start(priority=k % 2)

        def fetch_rows(src, dst, sem, i):
            for r in (0, 16):
                for q in range(2):
                    at = pl.ds(pl.multiple_of(i * 32 + r + q * (F // 2), 16), 16)
                    pltpu.make_async_copy(src.at[at, :], dst.at[at, :], sem).start(priority=q)

        def prep_wq(g):
            c = pl.ds(pl.multiple_of(g * G * DH, G * DH), G * DH)
            blk = wq_raw[:, c]
            wq[:, c] = pltpu.bitcast(blk, u32)
            csq[:, c] = jnp.dot(jnp.ones((16, D), bf16), blk, preferred_element_type=f32)[0:8]
            for j in range(VG):
                wqtf[g * VG + j] = blk[:, j * DH:(j + 1) * DH].T.astype(f32)

        def prep_wo(g):
            blk = wo_raw[pl.ds(pl.multiple_of(g * G * DH, G * DH), G * DH), :]
            wo[pl.ds(pl.multiple_of(g * G * 64, G * 64), G * 64), :] = pltpu.bitcast(blk, u32)
            for j in range(VG):
                wof[g * VG + j] = blk[j * DH:(j + 1) * DH].astype(f32)

        def prep_mlp(i):
            n = FP // 2
            r = pl.ds(pl.multiple_of(i * n, 128), n)
            blk = w1t_raw[r, :].T
            w1[:, r] = pltpu.bitcast(blk, u32)
            cs1[:, r] = jnp.dot(jnp.ones((16, D), bf16), blk, preferred_element_type=f32)[0:8]
            w2[pl.ds(pl.multiple_of(i * (n // 2), 64), n // 2), :] = pltpu.bitcast(w2_raw[r, :], u32)

        def prep_rest():
            b1v = jnp.concatenate([b1_raw[...].astype(f32)[None, :], jnp.zeros((1, FP - F), f32)], axis=1)
            b1[...] = jnp.broadcast_to(b1v, (8, FP))
            b2[...] = jnp.broadcast_to(b2_raw[...].astype(f32)[None, :], (8, D))

            def rows(i):
                r = pl.multiple_of(i * 64, 64)
                blk = w1t_raw[pl.ds(FM * 128 + r, 64), :].astype(f32)
                w1tf[pl.ds(r, 64), :] = blk
                cs1col[pl.ds(r, 64), :] = jnp.broadcast_to(jnp.sum(blk, axis=1, keepdims=True), (64, 128))
                w2f[pl.ds(r, 64), :] = w2_raw[pl.ds(FM * 128 + r, 64), :].astype(f32)
            loop(FV // 64, rows)
            for c in range(FM, FP // 128):
                n = min(128, F - c * 128)
                t = jnp.broadcast_to(b1v[:, c * 128:(c + 1) * 128], (128, 128)).T
                b1col[(c - FM) * 128:(c - FM) * 128 + n, :] = t[0:n]

        def prep_late(t):
            @pl.when(t == 0)
            def _():
                wait(w1t_raw.at[pl.ds(0, F), :], wsem.at[2])
                wait(w2_raw.at[pl.ds(0, F), :], wsem.at[3])
                w1t_raw[F:FP, :] = jnp.zeros((FP - F, D), bf16)
                w2_raw[F:FP, :] = jnp.zeros((FP - F, D), bf16)
            pl.when(t < 2)(lambda: prep_mlp(t))
            pl.when(t == 2)(prep_rest)

        loop(10, fetch_wq)
        small = [pltpu.make_async_copy(x_hbm, x_raw, wsem.at[4]),
                 pltpu.make_async_copy(b1_hbm, b1_raw, wsem.at[5]),
                 pltpu.make_async_copy(b2_hbm, b2_raw, wsem.at[6])]
        for cp in small:
            cp.start()
        loop(16, fetch_wo)
        loop(F // 64, lambda i: fetch_rows(w1t_hbm, w1t_raw, wsem.at[2], i))
        wait(wq_raw, wsem.at[0])

        def first_part(g):
            prep_wq(g)
            lax.fori_loop(7 * g, jnp.minimum(7 * g + 7, F // 64),
                          lambda i, c: (fetch_rows(w2_hbm, w2_raw, wsem.at[3], i), c)[1], 0)
        loop(NG, first_part)
        wait(wo_raw, wsem.at[1])

        def second_part(g):
            for i in range(2 * NS - BEHIND):
                pl.when(g == i * NG // (2 * NS - BEHIND))(lambda: stripe(i // NS, 0, i % NS))
            prep_wo(g)
        loop(NG, second_part)
        for cp in small:
            cp.wait()

        row = lax.broadcasted_iota(jnp.int32, (8, DH), 0)
        rowd = lax.broadcasted_iota(jnp.int32, (8, D), 0)
        xin[...] = x_raw[...].astype(f32)
        res[...] = jnp.zeros((8, D), f32)
        zero[...] = jnp.zeros((8, 128), jnp.int32)

        def start_layer(layer, x):
            xs[layer] = x
            accs[layer] = jnp.zeros((8, D), f32)

        def x_row(b):
            return jnp.broadcast_to(jnp.sum(jnp.where(rowd == b, xin[...], 0.0), axis=0, keepdims=True), (8, D))

        start_layer(0, x_row(0))

        def only_row(v, j):
            return unpack(pack(jnp.where(row == j, v, 0.0)))

        def queries(layer, g):
            c = pl.ds(pl.multiple_of(g * G * DH, G * DH), G * DH)
            x = xs[layer]
            m, var = moments(tiles(x))
            q = jnp.dot(jnp.concatenate([x, x], axis=0).astype(bf16), unpack(wq[:, c]),
                        preferred_element_type=f32)[0:8]
            return [t - m * cs for t, cs in zip(tiles(q), tiles(csq[:, c]))], lax.rsqrt(var + EPS) * SCALE

        def softmax(q, c, t, feed):
            s = None
            for j in range(G):
                feed()
                u = jnp.dot(only_row(q[j], j), unpack(kt[t % NV, j]), preferred_element_type=f32)[0:8]
                s = u if s is None else s + u
            s = tiles(s)
            mx = lane_max(tree(jnp.maximum, s))
            e = [jnp.exp2((u - mx) * c) for u in s]
            p = jnp.concatenate(e, axis=1)
            return jnp.concatenate([p, p], axis=0).astype(bf16), 1.0 / lane_sum(tree(jnp.add, e))

        def context(p, rl, t, js, feed=None):
            o = []
            for j in js:
                if feed:
                    feed()
                u = jnp.dot(p, unpack(v32[t % NV, j]), preferred_element_type=f32)[0:8]
                o.append(only_row(u * rl, j))
            r = ((t % NG) * G + js[0]) * 64
            r = r if isinstance(t, int) else pl.multiple_of(r, 64)
            return jnp.dot(jnp.concatenate(o, axis=1), unpack(wo[pl.ds(r, len(js) * 64), :]),
                           preferred_element_type=f32)[0:8]

        def transpose_v(t, js):
            for j in js:
                vtf[(t % NG) * VG + j] = unpack(v32[t % NV, j]).T.astype(f32)

        def after_attention(layer):
            return jnp.concatenate([a + row_sum(c) for a, c in zip(tiles(xs[layer]), tiles(accs[layer]))], axis=1)

        mlp_refs = (w1, w2, cs1, b1, b2, w1tf, w2f, b1col, cs1col)

        def step(t):
            g = t % NG

            lo = jnp.where(t > LAST - 2, t + 1, t)
            hi = jnp.where(t < NG, t, jnp.minimum(jnp.where(t >= LAST - 2, t + 2, t + 1), NPAGE))

            def second_layer(u, carry):
                feed = Feed(jnp.where(u == lo, t, NPAGE), 0, 2 * G + 1)
                feed()
                p, rl = softmax(*queries(1, u % NG), u - NG, feed)
                accs[1] += context(p, rl, u - NG, range(G), feed)
                return carry
            lax.fori_loop(lo, hi, second_layer, 0)

            @pl.when(t < NG)
            def _():
                Feed(t, 0, 1)()
                prep_late(t)

            feed = Feed(t, 1, 2 * G + 1)
            wait(kbuf.at[t % NK], ksem.at[t % NK])
            feed()
            q, c = queries(0, g)
            for j in range(G):
                feed()
                kj = unpack(k32[t % NK, j]).T
                kt[t % NV, j] = pltpu.bitcast(kj, u32)
                if j < VG:
                    ktf[g * VG + j] = kj.astype(f32)
            ps[t % 2], rls[t % 2] = softmax(q, c, t, feed)

            tc = jnp.minimum(t, LAST - 1)

            @pl.when(t != LAST - 1)
            def _():
                wait(vbuf.at[tc % NV], vsem.at[tc % NV])
                transpose_v(tc, range(VG))
                accs[0] += context(ps[tc % 2], rls[tc % 2], tc, range(G), Feed(t, 2, G))

            first = (g == NG - 1) & (t < LAST)
            second = ((g == 0) & (t >= 2 * NG)) | (t == LAST - 1)

            @pl.when((first & (t >= NG)) | (t == LAST - 1))
            def _():
                xs[2] = after_attention(1)

            @pl.when(first)
            def _():
                xs[0] = after_attention(0)

            @pl.when(first | second)
            def _():
                x = mlp(tiles(xs[jnp.where(first, 0, 2)]), mlp_refs, FP // 128, Feed(t, 3, 4))
                x = jnp.concatenate(x, axis=1)

                @pl.when(first)
                def _():
                    start_layer(1, x)
                    start_layer(0, x_row(t // NG + 1))

                @pl.when(second)
                def _():
                    res[...] = jnp.where(rowd == (t + 2) // NG - 2, x, res[...])

            @pl.when(jnp.logical_not(first | second) & (t < LAST))
            def _():
                Feed(t, 3, 1)()

        loop(NPAGE, step)

        p, rl = ps[LAST % 2], rls[LAST % 2]
        acc = accs[0]
        for i, (lo, hi) in enumerate(zip(LAST_CUTS[:-1], LAST_CUTS[1:])):
            wait(vbuf.at[LAST % NV, pl.ds(lo, hi - lo)], lsem.at[i])
            transpose_v(LAST, range(lo, min(hi, VPU_HEADS[-1])))
            acc = acc + context(p, rl, LAST, range(lo, hi))
        xt = [a + row_sum(c) for a, c in zip(tiles(xs[0]), tiles(acc))]
        always = zero[...] == 0

        def k_half(h, hf):
            return kt[(NPAGE - NG + h // G) % NV, h % G, :, hf * 512:(hf + 1) * 512]

        def v_half(h, hf):
            return v32[(NPAGE - NG + h // G) % NV, h % G, hf * 256:(hf + 1) * 256, :]

        xt = mlp(xt, mlp_refs, FM)
        xt = attention(xt, (k_half, v_half, wq, wo, csq, ktf, vtf, wqtf, wof), vheads, groups, always)
        xt = mlp(xt, mlp_refs, FM)
        o_ref[...] = jnp.where(rowd == B - 1, jnp.concatenate(xt, axis=1), res[...]).astype(o_ref.dtype)

    V = pltpu.VMEM
    scratch = [
        V((NK, G, W, DH), bf16), V((NV, G, W, DH), bf16), V((NV, G, DH // 2, W), u32),
        V((NG * VG, DH, W), f32), V((NG * VG, DH, W), f32),
        V((D, H * DH), bf16), V((H * DH, D), bf16), V((FP, D), bf16), V((FP, D), bf16),
        V((B, D), bf16), V((F,), bf16), V((D,), bf16),
        V((D // 2, H * DH), u32), V((H * DH // 2, D), u32), V((D // 2, FP), u32), V((FP // 2, D), u32),
        V((NG * VG, DH, D), f32), V((NG * VG, DH, D), f32), V((FV, D), f32), V((FV, D), f32),
        V((8, H * DH), f32), V((8, FP), f32), V((8, FP), f32), V((8, D), f32), V((FV, 128), f32), V((FV, 128), f32),
        V((8, D), f32), V((3, 8, D), f32), V((2, 8, D), f32), V((2, 16, W), bf16), V((2, 8, DH), f32),
        V((8, D), f32), V((8, 128), jnp.int32),
        pltpu.SemaphoreType.DMA((NK,)), pltpu.SemaphoreType.DMA((NV,)),
        pltpu.SemaphoreType.DMA((7,)), pltpu.SemaphoreType.DMA((len(LAST_CUTS) - 1,)),
    ]

    return kernel, scratch


@jax.jit
def pallas_interleave_layers__sliding_block_cached__mixer_channel_mlp__decode_kernel(
    A_x: jax.Array,
    A_k_cache: jax.Array,
    A_v_cache: jax.Array,
    A_wq: jax.Array,
    A_wo: jax.Array,
    B_x: jax.Array,
    B_w1: jax.Array,
    B_b1: jax.Array,
    B_w2: jax.Array,
    B_b2: jax.Array,
):
    del B_x
    kernel, scratch = build_kernel()
    out = pl.pallas_call(
        kernel,
        in_specs=[pl.BlockSpec(memory_space=pltpu.HBM)] * 9,
        out_specs=pl.BlockSpec(memory_space=pltpu.VMEM),
        out_shape=jax.ShapeDtypeStruct((B, D), A_x.dtype),
        scratch_shapes=scratch,
        compiler_params=pltpu.CompilerParams(vmem_limit_bytes=112 * 1024 * 1024, disable_bounds_checks=True),
    )(A_x.reshape(B, D), A_k_cache, A_v_cache, A_wq, A_wo, B_w1.T, B_b1, B_w2, B_b2)
    return out.reshape(B, 1, D)
```

```python
import jax
import jax.numpy as jnp
from jax import lax
from jax.experimental import pallas as pl
from jax.experimental.pallas import tpu as pltpu

B, D, H, DH, SK, F = 8, 640, 32, 128, 4096, 1728
W = min(4096, max(256, SK // 4))
FP = 1792
DT = D // 128
G = 8
NG = H // G
NPAGE = B * NG
NK, NV = 4, 8
EPS = 1e-5
SCALE = DH ** -0.5 * 1.4426950408889634

LAST = NPAGE - 1

PIECE_ROWS = (64, 96) * 6 + (64,)
NS = len(PIECE_ROWS)
HEAD_ORDER = (0, 4, 3, 7, 6, 2, 1, 5)
REGIONS = (0, 4, 1, 5, 2, 6, 3, 7)
BEHIND = 5
FEED = (0, 9, 19, 21, 2 * NS)
LAST_SLOTS = [(LAST - 1, i) for i in range(21, 26)] + [(LAST, i) for i in range(9, 17)]
LAST_CUTS = (0, 6, 8)

VG = 3
MXU_GROUPS = (4, 8, 8)
FM = 10
FV = F - FM * 128
JB = 4

f32, bf16, u32 = jnp.float32, jnp.bfloat16, jnp.uint32


def tiles(v):
    return [v[:, i * 128:(i + 1) * 128] for i in range(v.shape[1] // 128)]


def tree(op, xs):
    xs = list(xs)
    while len(xs) > 1:
        xs = [op(*xs[i:i + 2]) if i + 1 < len(xs) else xs[i] for i in range(0, len(xs), 2)]
    return xs[0]


def lane_sum(v):
    return jnp.broadcast_to(jnp.sum(v, axis=1, keepdims=True), v.shape)


def lane_max(v):
    return jnp.broadcast_to(jnp.max(v, axis=1, keepdims=True), v.shape)


def row_sum(v):
    return jnp.broadcast_to(jnp.sum(v, axis=0, keepdims=True), v.shape)


def accum(acc, i, val):
    acc[i] = val if acc[i] is None else acc[i] + val


def pack(a, b=None):
    return pltpu.bitcast(jnp.concatenate([a, a if b is None else b], axis=0).astype(bf16), u32)


def unpack(w):
    return pltpu.bitcast(w, bf16)


def mxu_dot(lhs, w, half=0):
    lhs = jnp.concatenate([unpack(t) for t in lhs], axis=1)
    return jnp.dot(lhs, unpack(w), preferred_element_type=f32)[half * 8:half * 8 + 8]


def moments(xt):
    m = lane_sum(tree(jnp.add, xt)) * (1.0 / D)
    sq = lane_sum(tree(jnp.add, [t * t for t in xt])) * (1.0 / D)
    return m, jnp.maximum(sq - m * m, 0.0)


def gelu(x):
    c = 0.7978845608028654
    hx = 0.5 * x
    return hx + hx * jnp.tanh(x * (c + (c * 0.044715) * (x * x)))


def loop(n, body):
    lax.fori_loop(0, n, lambda i, c: (body(i), c)[1], 0)


class Weave:
    def __init__(self, always=None, lag_m=3, lag_v=4):
        self.always, self.lag_m, self.lag_v = always, lag_m, lag_v
        self.vres, self.mres, self.fresh = [], [], False

    def tie_m(self, lhs):
        k = len(self.mres) - self.lag_m
        if k < 0 or self.vres[k] is None:
            return lhs
        return jnp.where(self.always, lhs, pltpu.bitcast(self.vres[k], u32))

    def tie_v(self, val):
        k = len(self.mres) - self.lag_v
        if k < 0 or not self.fresh:
            return val
        self.fresh = False
        return jnp.where(self.always, val, self.mres[k])

    def run(self, mxu, mxu_work, vpu, vpu_work):
        md = vd = 0
        last = None
        mxu_live, vpu_live = True, vpu_work > 0
        while mxu_live or vpu_live:
            if mxu_live and (not vpu_live or md * vpu_work <= vd * mxu_work):
                item = next(mxu, None)
                mxu_live = item is not None
                if mxu_live:
                    md += item[0]
                    self.vres.append(last)
                    self.mres.append(item[1])
                    self.fresh = True
            else:
                item = next(vpu, None)
                vpu_live = item is not None
                if vpu_live:
                    vd += item[0]
                    last = item[1]


def mlp(xt, refs, fm, feed=None):
    w1, w2, cs1, b1, b2, w1tf, w2f, b1col, cs1col = refs
    m1 = lane_sum(tree(jnp.add, xt)) * (1.0 / D)
    xc = [t - m1 for t in xt]
    mc, vc = moments(xc)
    r1 = lax.rsqrt(vc + mc * mc + EPS)
    r2 = lax.rsqrt(vc * r1 * r1 + EPS)
    m, r = m1 + mc, r1 * r2
    xp = [pack(xt[i], xt[min(i + 1, DT - 1)]) for i in range(0, DT, 2)]
    macc, vacc = [None] * DT, [None] * DT
    chunks = [(c, min(4, fm - c)) for c in range(0, fm, 4)]
    nj = max(F - fm * 128, 0) // 8

    def mxu():
        hs = {}

        def up(i):
            c0, n = chunks[i]
            a = None
            for kb in range(DT):
                u = mxu_dot([xp[kb // 2]], w1[kb * 64:(kb + 1) * 64, c0 * 128:(c0 + n) * 128], kb % 2)
                a = u if a is None else a + u
                yield 8 * n, None
            hs[i] = []
            for j, t in enumerate(tiles(a)):
                sl = slice((c0 + j) * 128, (c0 + j + 1) * 128)
                hs[i].append(pack(gelu((t - m * cs1[:, sl]) * r + b1[:, sl])))

        def down(i):
            c0, n = chunks[i]
            for nt in range(DT):
                accum(macc, nt, mxu_dot(hs[i], w2[c0 * 64:(c0 + n) * 64, nt * 128:(nt + 1) * 128]))
                yield 8 * n, None

        for t in range(len(chunks) + 1):
            if t < len(chunks):
                if feed:
                    feed()
                yield from up(t)
            if t >= 1:
                yield from down(t - 1)

    def vpu():
        delay = 48
        col, part = {}, {}
        for step in range(nj + delay):
            if step < nj:
                blk, sub = divmod(step, JB)
                js = range(blk * JB, (blk + 1) * JB)
                for kb in range(DT):
                    if kb * JB // DT == sub:
                        for j in js:
                            t = w1tf[j * 8:(j + 1) * 8, kb * 128:(kb + 1) * 128] * xc[kb]
                            part[j] = t if kb == 0 else part[j] + t
                        yield JB, None
                if sub == JB - 1:
                    for j in js:
                        col[j] = lane_sum(part.pop(j))
            j = step - delay
            if j >= 0:
                sl = slice(j * 8, (j + 1) * 8)
                h = gelu((col.pop(j) - mc * cs1col[sl, :]) * r + b1col[sl, :])
                for nt in range(DT):
                    accum(vacc, nt, w2f[j * 8:(j + 1) * 8, nt * 128:(nt + 1) * 128] * h)
                yield 5, None

    Weave().run(mxu(), fm * 80, vpu(), nj * 10)
    out = []
    for nt in range(DT):
        a = xt[nt] + b2[:, nt * 128:(nt + 1) * 128] + macc[nt]
        out.append(a if vacc[nt] is None else a + row_sum(vacc[nt]))
    return out


def attention(xt, refs, vheads, groups, always):
    k_half, v_half, wq, wo, csq, ktf, vtf, wqtf, wof = refs
    weave = Weave(always)
    row = lax.broadcasted_iota(jnp.int32, (8, DH), 0)
    m, var = moments(xt)
    c = lax.rsqrt(var + EPS) * SCALE
    xc = [t - m for t in xt]
    xp = [pack(xt[i], xt[min(i + 1, DT - 1)]) for i in range(0, DT, 2)]
    macc, vacc = [None] * DT, [None] * DT

    def mxu():
        q, p, o = {}, {}, {}

        def project(g):
            for c0 in range(0, len(groups[g]), 4):
                hs = groups[g][c0:c0 + 4]
                a = None
                for kb in range(DT):
                    w = jnp.concatenate([wq[kb * 64:(kb + 1) * 64, h * 128:(h + 1) * 128] for h in hs], axis=1)
                    u = mxu_dot([weave.tie_m(xp[kb // 2])], w, kb % 2)
                    a = u if a is None else a + u
                    yield 8 * len(hs), u[:, 0:128]
                for i, t in enumerate(tiles(a)):
                    t = t - m * csq[:, hs[i] * 128:(hs[i] + 1) * 128]
                    q[g] = jnp.where(row == c0 + i, t, q[g]) if g in q else t

        def scores(g):
            s = [None] * 8
            for hf in range(2):
                for j, h in enumerate(groups[g]):
                    u = mxu_dot([weave.tie_m(pack(jnp.where(row == j, q[g], 0.0)))], k_half(h, hf))
                    for i, t in enumerate(tiles(u)):
                        accum(s, hf * 4 + i, t)
                    yield 32, u[:, 0:128]
            mx = lane_max(tree(jnp.maximum, s))
            e = [jnp.exp2((t - mx) * c) for t in s]
            p[g] = ([pack(e[i], e[i + 4]) for i in range(4)], 1.0 / lane_sum(tree(jnp.add, e)))

        def context(g):
            pk, rl = p[g]
            out = None
            for j, h in enumerate(groups[g]):
                a = None
                for hf in range(2):
                    u = mxu_dot([weave.tie_m(pk[0])] + pk[1:], v_half(h, hf), hf)
                    a = u if a is None else a + u
                    yield 32, u
                out = a if out is None else jnp.where(row == j, a, out)
            o[g] = out * rl

        def output(g):
            for c0 in range(0, len(groups[g]), 4):
                hs = groups[g][c0:c0 + 4]
                lhs = [pack(jnp.where(row == c0 + i, o[g], 0.0)) for i in range(len(hs))]
                for nt in range(DT):
                    w = jnp.concatenate([wo[h * 64:(h + 1) * 64, nt * 128:(nt + 1) * 128] for h in hs], axis=0)
                    u = mxu_dot([weave.tie_m(lhs[0])] + lhs[1:], w)
                    accum(macc, nt, u)
                    yield 8 * len(hs), u

        for t in range(len(groups) + 3):
            for d, stage in enumerate((project, scores, context, output)):
                if 0 <= t - d < len(groups):
                    yield from stage(t - d)

    def vpu():
        qcol, ocol, s, e, rl, qa, oa, seen = {}, {}, {}, {}, {}, {}, {}, {}

        def fold_rows(vals):
            low = (row & 4) == 0
            vals = [jnp.where(low, vals[k], vals[k + 4]) + pltpu.roll(jnp.where(low, vals[k + 4], vals[k]), 4, 0)
                    for k in range(4)]
            for sh in (2, 1):
                low = (row & sh) == 0
                vals = [jnp.where(low, vals[k] + pltpu.roll(vals[k], 8 - sh, 0),
                                  vals[k + sh] + pltpu.roll(vals[k + sh], sh, 0)) for k in range(sh)]
            return vals[0]

        def project(i):
            h, blk, sub = vheads[i // 16], (i % 16) // JB, i % JB
            js = range(blk * JB, (blk + 1) * JB)
            for kb in range(DT):
                if kb * JB // DT == sub:
                    x0 = weave.tie_v(xc[kb])
                    for j in js:
                        t = wqtf[h, j * 8:(j + 1) * 8, kb * 128:(kb + 1) * 128] * x0
                        qa[j] = t if kb == 0 else qa[j] + t
                    yield JB, qa[j]
            if sub == JB - 1:
                for j in js:
                    qcol[i // 16 * 16 + j] = lane_sum(qa[j])

        def scores(i):
            h, j = vheads[i // 16], i % 16
            sa = s.setdefault(h, [None] * 8)
            qc = weave.tie_v(qcol.pop(i))
            if i - 2 in seen:
                qc = jnp.where(always, qc, seen.pop(i - 2))
            for t in range(8):
                accum(sa, t, ktf[h, j * 8:(j + 1) * 8, t * 128:(t + 1) * 128] * qc)
            seen[i] = sa[0]
            if j == 15:
                sc = fold_rows(s.pop(h))
                mx = lane_max(jnp.broadcast_to(jnp.max(sc, axis=0, keepdims=True), sc.shape))
                e[h] = jnp.exp2((sc - mx) * c)
                rl[h] = 1.0 / lane_sum(row_sum(e[h]))
            yield 8, sa[7]

        def context(i):
            h, blk, sub = vheads[i // 16], (i % 16) // JB, i % JB
            js = range(blk * JB, (blk + 1) * JB)
            for t in range(8):
                if t * JB // 8 == sub:
                    e0 = weave.tie_v(jnp.broadcast_to(e[h][t:t + 1, :], (8, DH)))
                    for j in js:
                        u = vtf[h, j * 8:(j + 1) * 8, t * 128:(t + 1) * 128] * e0
                        oa[j] = u if t == 0 else oa[j] + u
                    yield JB, oa[j]
            if sub == JB - 1:
                for j in js:
                    ocol[i // 16 * 16 + j] = lane_sum(oa[j]) * rl[h]

        def output(i):
            h, j = vheads[i // 16], i % 16
            oc = weave.tie_v(ocol.pop(i))
            for nt in range(DT):
                accum(vacc, nt, wof[h, j * 8:(j + 1) * 8, nt * 128:(nt + 1) * 128] * oc)
            yield 5, vacc[DT - 1]

        n = len(vheads) * 16
        stages = ((project, 0), (scores, 12), (context, 38), (output, 48))
        for step in range(n + stages[-1][1]):
            for stage, delay in stages:
                if 0 <= step - delay < n:
                    yield from stage(step - delay)

    weave.run(mxu(), sum(len(g) for g in groups) * 208, vpu(), len(vheads) * 416)
    return [xt[nt] + row_sum(macc[nt] + vacc[nt]) for nt in range(DT)]


def build_kernel():
    vheads = [g * VG + j for g in range(NG) for j in range(VG)]
    mheads = [g * G + j for g in range(NG) for j in range(VG, G)]
    groups = [mheads[sum(MXU_GROUPS[:i]):sum(MXU_GROUPS[:i + 1])] for i in range(len(MXU_GROUPS))]

    def kernel(x_hbm, k_hbm, v_hbm, wq_hbm, wo_hbm, w1t_hbm, b1_hbm, w2_hbm, b2_hbm, o_ref,
               kbuf, vbuf, kt, vp, ktf, vtf,
               wq_raw, wo_raw, w1t_raw, w2_raw, x_raw, b1_raw, b2_raw,
               wq, wo, w1, w2, wqtf, wof, w1tf, w2f, csq, cs1, b1, b2, b1col, cs1col,
               xin, xs, accs, ps, rls, res, zero, ksem, vsem, wsem, lsem):
        def piece(src, buf, sem, t, hh, n, queue):
            r, size = sum(PIECE_ROWS[:n]), PIECE_ROWS[n]
            pltpu.make_async_copy(
                src.at[t // NG, (t % NG) * G + hh, pl.ds(SK - W + r, size), :],
                buf.at[t % buf.shape[0], hh, pl.ds(r, size), :], sem).start(priority=queue)

        def stripe(is_v, t, n):
            src, buf, sem = ((k_hbm, kbuf, ksem), (v_hbm, vbuf, vsem))[is_v]
            for i, hh in enumerate(HEAD_ORDER):
                piece(src, buf, sem.at[t % buf.shape[0]], t, hh, n, i % 2)

        def last_stripe(i):
            order = [(h + k * (G // 2), n) for h in range(G // 2) for n in range(NS) for k in range(2)]
            for hh, n in order[i * G:(i + 1) * G]:
                part = sum(hh >= c for c in LAST_CUTS[1:-1])
                piece(v_hbm, vbuf, lsem.at[part], LAST, hh, n, hh // (G // 2))

        def slot(t, i):
            for n, (tt, ii) in enumerate(LAST_SLOTS):
                if ii == i:
                    pl.when(t == tt)(lambda: last_stripe(n))
            wrap, i = divmod(i - BEHIND, 2 * NS)
            is_v, n = divmod(i, NS)
            page = t + 1 + wrap
            swapped = LAST - is_v
            pl.when(page < swapped)(lambda: stripe(is_v, page, n))
            pl.when(page == swapped)(lambda: stripe(1 - is_v, LAST - 1 + is_v, n))

        class Feed:
            def __init__(self, t, part, calls):
                self.t, self.lo, self.n, self.calls, self.k = t, FEED[part], FEED[part + 1] - FEED[part], calls, 0

            def __call__(self):
                a, e = (self.lo - (-self.n * k // self.calls) for k in (self.k, self.k + 1))
                self.k += 1
                for i in range(a, e):
                    slot(self.t, i)

        def wait(ref, sem):
            pltpu.make_async_copy(ref, ref, sem).wait()

        def fetch_wq(i):
            c = 0
            for n in (8 * 128, 12 * 128, 12 * 128):
                for k, h in enumerate(REGIONS):
                    at = (pl.ds(pl.multiple_of((h * 10 + i) * 8, 8), 8), pl.ds(c, n))
                    pltpu.make_async_copy(wq_hbm.at[at], wq_raw.at[at], wsem.at[0]).start(priority=k % 2)
                c += n

        def fetch_wo(i):
            for r, n in ((0, 8), (8, 24)):
                for k, h in enumerate(REGIONS):
                    at = pl.ds(pl.multiple_of(h * 512 + i * 32 + r, 8), n)
                    pltpu.make_async_copy(wo_hbm.at[at, :], wo_raw.at[at, :], wsem.at[1]).start(priority=k % 2)

        def fetch_rows(src, dst, sem, i):
            for r in (0, 16):
                for q in range(2):
                    at = pl.ds(pl.multiple_of(i * 32 + r + q * (F // 2), 16), 16)
                    pltpu.make_async_copy(src.at[at, :], dst.at[at, :], sem).start(priority=q)

        def prep_wq(g):
            c = pl.ds(pl.multiple_of(g * G * DH, G * DH), G * DH)
            blk = wq_raw[:, c]
            wq[:, c] = pltpu.bitcast(blk, u32)
            csq[:, c] = jnp.dot(jnp.ones((16, D), bf16), blk, preferred_element_type=f32)[0:8]
            for j in range(VG):
                wqtf[g * VG + j] = blk[:, j * DH:(j + 1) * DH].T.astype(f32)

        def prep_wo(g):
            blk = wo_raw[pl.ds(pl.multiple_of(g * G * DH, G * DH), G * DH), :]
            wo[pl.ds(pl.multiple_of(g * G * 64, G * 64), G * 64), :] = pltpu.bitcast(blk, u32)
            for j in range(VG):
                wof[g * VG + j] = blk[j * DH:(j + 1) * DH].astype(f32)

        def prep_mlp(i):
            n = FP // 2
            r = pl.ds(pl.multiple_of(i * n, 128), n)
            blk = w1t_raw[r, :].T
            w1[:, r] = pltpu.bitcast(blk, u32)
            cs1[:, r] = jnp.dot(jnp.ones((16, D), bf16), blk, preferred_element_type=f32)[0:8]
            w2[pl.ds(pl.multiple_of(i * (n // 2), 64), n // 2), :] = pltpu.bitcast(w2_raw[r, :], u32)

        def prep_rest():
            b1v = jnp.concatenate([b1_raw[...].astype(f32)[None, :], jnp.zeros((1, FP - F), f32)], axis=1)
            b1[...] = jnp.broadcast_to(b1v, (8, FP))
            b2[...] = jnp.broadcast_to(b2_raw[...].astype(f32)[None, :], (8, D))

            def rows(i):
                r = pl.multiple_of(i * 64, 64)
                blk = w1t_raw[pl.ds(FM * 128 + r, 64), :].astype(f32)
                w1tf[pl.ds(r, 64), :] = blk
                cs1col[pl.ds(r, 64), :] = jnp.broadcast_to(jnp.sum(blk, axis=1, keepdims=True), (64, 128))
                w2f[pl.ds(r, 64), :] = w2_raw[pl.ds(FM * 128 + r, 64), :].astype(f32)
            loop(FV // 64, rows)
            for c in range(FM, FP // 128):
                n = min(128, F - c * 128)
                t = jnp.broadcast_to(b1v[:, c * 128:(c + 1) * 128], (128, 128)).T
                b1col[(c - FM) * 128:(c - FM) * 128 + n, :] = t[0:n]

        def prep_late(t):
            @pl.when(t == 0)
            def _():
                wait(w1t_raw.at[pl.ds(0, F), :], wsem.at[2])
                wait(w2_raw.at[pl.ds(0, F), :], wsem.at[3])
                w1t_raw[F:FP, :] = jnp.zeros((FP - F, D), bf16)
                w2_raw[F:FP, :] = jnp.zeros((FP - F, D), bf16)
            pl.when(t < 2)(lambda: prep_mlp(t))
            pl.when(t == 2)(prep_rest)

        loop(10, fetch_wq)
        small = [pltpu.make_async_copy(x_hbm, x_raw, wsem.at[4]),
                 pltpu.make_async_copy(b1_hbm, b1_raw, wsem.at[5]),
                 pltpu.make_async_copy(b2_hbm, b2_raw, wsem.at[6])]
        for cp in small:
            cp.start()
        loop(16, fetch_wo)
        loop(F // 64, lambda i: fetch_rows(w1t_hbm, w1t_raw, wsem.at[2], i))
        wait(wq_raw, wsem.at[0])

        def first_part(g):
            prep_wq(g)
            lax.fori_loop(7 * g, jnp.minimum(7 * g + 7, F // 64),
                          lambda i, c: (fetch_rows(w2_hbm, w2_raw, wsem.at[3], i), c)[1], 0)
        loop(NG, first_part)
        wait(wo_raw, wsem.at[1])

        def second_part(g):
            for i in range(2 * NS - BEHIND):
                pl.when(g == i * NG // (2 * NS - BEHIND))(lambda: stripe(i // NS, 0, i % NS))
            prep_wo(g)
        loop(NG, second_part)
        for cp in small:
            cp.wait()

        row = lax.broadcasted_iota(jnp.int32, (8, DH), 0)
        rowd = lax.broadcasted_iota(jnp.int32, (8, D), 0)
        xin[...] = x_raw[...].astype(f32)
        res[...] = jnp.zeros((8, D), f32)
        zero[...] = jnp.zeros((8, 128), jnp.int32)

        def start_layer(layer, x):
            xs[layer] = x
            accs[layer] = jnp.zeros((8, D), f32)

        def x_row(b):
            return jnp.broadcast_to(jnp.sum(jnp.where(rowd == b, xin[...], 0.0), axis=0, keepdims=True), (8, D))

        start_layer(0, x_row(0))

        def only_row(v, j):
            return unpack(pack(jnp.where(row == j, v, 0.0)))

        def queries(layer, g):
            c = pl.ds(pl.multiple_of(g * G * DH, G * DH), G * DH)
            x = xs[layer]
            m, var = moments(tiles(x))
            q = jnp.dot(jnp.concatenate([x, x], axis=0).astype(bf16), unpack(wq[:, c]),
                        preferred_element_type=f32)[0:8]
            return [t - m * cs for t, cs in zip(tiles(q), tiles(csq[:, c]))], lax.rsqrt(var + EPS) * SCALE

        def softmax(q, c, t, feed):
            s = None
            for j in range(G):
                feed()
                u = jnp.dot(only_row(q[j], j), unpack(kt[t % NV, j]), preferred_element_type=f32)[0:8]
                s = u if s is None else s + u
            s = tiles(s)
            mx = lane_max(tree(jnp.maximum, s))
            e = [jnp.exp2((u - mx) * c) for u in s]
            p = jnp.concatenate(e, axis=1)
            return jnp.concatenate([p, p], axis=0).astype(bf16), 1.0 / lane_sum(tree(jnp.add, e))

        def context(p, rl, t, js, feed=None, keep=False):
            o = []
            for j in js:
                if feed:
                    feed()
                vj = vbuf[t % NV, j]
                if keep and j >= VG:
                    vp[t % NG, j - VG] = pltpu.bitcast(vj, u32)
                u = jnp.dot(p, vj, preferred_element_type=f32)[0:8]
                o.append(only_row(u * rl, j))
            r = ((t % NG) * G + js[0]) * 64
            r = r if isinstance(t, int) else pl.multiple_of(r, 64)
            return jnp.dot(jnp.concatenate(o, axis=1), unpack(wo[pl.ds(r, len(js) * 64), :]),
                           preferred_element_type=f32)[0:8]

        def transpose_v(t, js):
            for j in js:
                vtf[(t % NG) * VG + j] = vbuf[t % NV, j].T.astype(f32)

        def after_attention(layer):
            return jnp.concatenate([a + row_sum(c) for a, c in zip(tiles(xs[layer]), tiles(accs[layer]))], axis=1)

        mlp_refs = (w1, w2, cs1, b1, b2, w1tf, w2f, b1col, cs1col)

        def step(t):
            g = t % NG

            lo = jnp.where(t > LAST - 2, t + 1, t)
            hi = jnp.where(t < NG, t, jnp.minimum(jnp.where(t >= LAST - 2, t + 2, t + 1), NPAGE))

            def second_layer(u, carry):
                feed = Feed(jnp.where(u == lo, t, NPAGE), 0, 2 * G + 1)
                feed()
                p, rl = softmax(*queries(1, u % NG), u - NG, feed)
                accs[1] += context(p, rl, u - NG, range(G), feed)
                return carry
            lax.fori_loop(lo, hi, second_layer, 0)

            @pl.when(t < NG)
            def _():
                Feed(t, 0, 1)()
                prep_late(t)

            feed = Feed(t, 1, 2 * G + 1)
            wait(kbuf.at[t % NK], ksem.at[t % NK])
            feed()
            q, c = queries(0, g)
            for j in range(G):
                feed()
                kj = kbuf[t % NK, j].T
                kt[t % NV, j] = pltpu.bitcast(kj, u32)
                if j < VG:
                    ktf[g * VG + j] = kj.astype(f32)
            ps[t % 2], rls[t % 2] = softmax(q, c, t, feed)

            tc = jnp.minimum(t, LAST - 1)

            @pl.when(t != LAST - 1)
            def _():
                wait(vbuf.at[tc % NV], vsem.at[tc % NV])
                transpose_v(tc, range(VG))
                accs[0] += context(ps[tc % 2], rls[tc % 2], tc, range(G), Feed(t, 2, G), keep=True)

            first = (g == NG - 1) & (t < LAST)
            second = ((g == 0) & (t >= 2 * NG)) | (t == LAST - 1)

            @pl.when((first & (t >= NG)) | (t == LAST - 1))
            def _():
                xs[2] = after_attention(1)

            @pl.when(first)
            def _():
                xs[0] = after_attention(0)

            @pl.when(first | second)
            def _():
                x = mlp(tiles(xs[jnp.where(first, 0, 2)]), mlp_refs, FP // 128, Feed(t, 3, 4))
                x = jnp.concatenate(x, axis=1)

                @pl.when(first)
                def _():
                    start_layer(1, x)
                    start_layer(0, x_row(t // NG + 1))

                @pl.when(second)
                def _():
                    res[...] = jnp.where(rowd == (t + 2) // NG - 2, x, res[...])

            @pl.when(jnp.logical_not(first | second) & (t < LAST))
            def _():
                Feed(t, 3, 1)()

        loop(NPAGE, step)

        p, rl = ps[LAST % 2], rls[LAST % 2]
        acc = accs[0]
        for i, (lo, hi) in enumerate(zip(LAST_CUTS[:-1], LAST_CUTS[1:])):
            wait(vbuf.at[LAST % NV, pl.ds(lo, hi - lo)], lsem.at[i])
            transpose_v(LAST, range(lo, min(hi, VG)))
            acc = acc + context(p, rl, LAST, range(lo, hi), keep=hi < G)
        xt = [a + row_sum(c) for a, c in zip(tiles(xs[0]), tiles(acc))]
        always = zero[...] == 0

        def k_half(h, hf):
            return kt[(NPAGE - NG + h // G) % NV, h % G, :, hf * 512:(hf + 1) * 512]

        def v_half(h, hf):
            if h >= H - G + LAST_CUTS[-2]:
                return pltpu.bitcast(vbuf[LAST % NV, h % G, hf * 512:(hf + 1) * 512, :], u32)
            return vp[h // G, h % G - VG, hf * 256:(hf + 1) * 256, :]

        xt = mlp(xt, mlp_refs, FM)
        xt = attention(xt, (k_half, v_half, wq, wo, csq, ktf, vtf, wqtf, wof), vheads, groups, always)
        xt = mlp(xt, mlp_refs, FM)
        o_ref[...] = jnp.where(rowd == B - 1, jnp.concatenate(xt, axis=1), res[...]).astype(o_ref.dtype)

    V = pltpu.VMEM
    scratch = [
        V((NK, G, W, DH), bf16), V((NV, G, W, DH), bf16), V((NV, G, DH // 2, W), u32),
        V((NG, G - VG, W // 2, DH), u32),
        V((NG * VG, DH, W), f32), V((NG * VG, DH, W), f32),
        V((D, H * DH), bf16), V((H * DH, D), bf16), V((FP, D), bf16), V((FP, D), bf16),
        V((B, D), bf16), V((F,), bf16), V((D,), bf16),
        V((D // 2, H * DH), u32), V((H * DH // 2, D), u32), V((D // 2, FP), u32), V((FP // 2, D), u32),
        V((NG * VG, DH, D), f32), V((NG * VG, DH, D), f32), V((FV, D), f32), V((FV, D), f32),
        V((8, H * DH), f32), V((8, FP), f32), V((8, FP), f32), V((8, D), f32), V((FV, 128), f32), V((FV, 128), f32),
        V((8, D), f32), V((3, 8, D), f32), V((2, 8, D), f32), V((2, 16, W), bf16), V((2, 8, DH), f32),
        V((8, D), f32), V((8, 128), jnp.int32),
        pltpu.SemaphoreType.DMA((NK,)), pltpu.SemaphoreType.DMA((NV,)),
        pltpu.SemaphoreType.DMA((7,)), pltpu.SemaphoreType.DMA((len(LAST_CUTS) - 1,)),
    ]

    return kernel, scratch


@jax.jit
def pallas_interleave_layers__sliding_block_cached__mixer_channel_mlp__decode_kernel(
    A_x: jax.Array,
    A_k_cache: jax.Array,
    A_v_cache: jax.Array,
    A_wq: jax.Array,
    A_wo: jax.Array,
    B_x: jax.Array,
    B_w1: jax.Array,
    B_b1: jax.Array,
    B_w2: jax.Array,
    B_b2: jax.Array,
):
    del B_x
    kernel, scratch = build_kernel()
    out = pl.pallas_call(
        kernel,
        in_specs=[pl.BlockSpec(memory_space=pltpu.HBM)] * 9,
        out_specs=pl.BlockSpec(memory_space=pltpu.VMEM),
        out_shape=jax.ShapeDtypeStruct((B, D), A_x.dtype),
        scratch_shapes=scratch,
        compiler_params=pltpu.CompilerParams(vmem_limit_bytes=112 * 1024 * 1024, disable_bounds_checks=True),
    )(A_x.reshape(B, D), A_k_cache, A_v_cache, A_wq, A_wo, B_w1.T, B_b1, B_w2, B_b2)
    return out.reshape(B, 1, D)
```
